```python
import os as _os
_os.environ.setdefault("JAX_PLATFORMS", "cpu")
import jax
import jax.numpy as jnp

def _softmax(x, axis=-1):
    return jax.nn.softmax(x, axis=axis)
def _gelu(x):
    return jax.nn.gelu(x, approximate=True)
def _silu(x):
    return jax.nn.silu(x)
def _sigmoid(x):
    return jax.nn.sigmoid(x)
def _layernorm(x, axis=-1, eps=1e-5):
    m = jnp.mean(x, axis=axis, keepdims=True)
    v = jnp.var(x, axis=axis, keepdims=True)
    return (x - m) / jnp.sqrt(v + eps)
def _scatter_add(tgt, idx, src, axis=0):
    return tgt.at[idx].add(src)
def _segment_sum(src, seg, n):
    return jax.ops.segment_sum(src, seg, n)
class _Rng:
    def __init__(self, key):
        self._k = key
    def _next(self):
        self._k, sub = jax.random.split(self._k)
        return sub
    def normal(self, shape):
        return jax.random.normal(self._next(), shape, dtype=jnp.bfloat16)
    def randint(self, lo, hi, shape):
        return jax.random.randint(self._next(), shape, lo, hi, dtype=jnp.int32)
    def uniform(self, shape, lo=0.0, hi=1.0):
        return jax.random.uniform(self._next(), shape, jnp.bfloat16, lo, hi)
    def permutation(self, n):
        return jax.random.permutation(self._next(), n)


kernel_name = 'parallel_sum__grouped_kv_mqa__dense_activation_silu__prompt'

def setup_inputs():
    _rng = _Rng(jax.random.key(int.from_bytes(__import__("os").urandom(4), "little")))
    _w = (lambda a: (lambda t: t.astype(jnp.bfloat16) if jnp.issubdtype(t.dtype, jnp.floating) else t)(jnp.asarray(a)))
    def _A_setup():
        B, S, D, H = 1, 2048, 512, 32
        Dh = D // H
        return {
            "x": _w((lambda *s: _rng.normal(s) * 0.05)(B, S, D)),
            "wq": _w((lambda *s: _rng.normal(s) * 0.05)(D, H * Dh)),
            "wk": _w((lambda *s: _rng.normal(s) * 0.05)(D, Dh)),
            "wv": _w((lambda *s: _rng.normal(s) * 0.05)(D, Dh)),
            "wo": _w((lambda *s: _rng.normal(s) * 0.05)(H * Dh, D)),
        }
    _A_in = _A_setup()

    def _B_setup():
        B, S, D, F = 1, 2048, 512, 1792
        return {
            "x": _w((lambda *s: _rng.normal(s) * 0.05)(B, S, D)),
            "w1": _w((lambda *s: _rng.normal(s) * 0.05)(D, F) * (D ** -0.5)),
            "w2": _w((lambda *s: _rng.normal(s) * 0.05)(F, D) * (F ** -0.5)),
        }
    _B_in = _B_setup()

    return {
        "A_x": _A_in["x"],
        "A_wq": _A_in["wq"],
        "A_wk": _A_in["wk"],
        "A_wv": _A_in["wv"],
        "A_wo": _A_in["wo"],
        "B_x": _B_in["x"],
        "B_w1": _B_in["w1"],
        "B_w2": _B_in["w2"],
    }

def reference(A_x, A_wq, A_wk, A_wv, A_wo, B_x, B_w1, B_w2):
    def _A_ref(x, wq, wk, wv, wo):
        B, S, D = x.shape
        H = 32
        Dh = D // H
        q = (lambda x, *d: x.transpose(*d))((x @ wq).reshape(B, S, H, Dh), 0, 2, 1, 3)
        k = x @ wk
        v = x @ wv
        scores = jnp.einsum("bhqd,bkd->bhqk", q, k) * (Dh ** -0.5)
        p = _softmax(scores, axis=-1)
        o = jnp.einsum("bhqk,bkd->bhqd", p, v)
        return (lambda x, *d: x.transpose(*d))(o, 0, 2, 1, 3).reshape(B, S, H * Dh) @ wo

    def _B_ref(x, w1, w2):
        h = jnp.einsum("bsd,df->bsf", x, w1)
        h = _silu(h)
        out = jnp.einsum("bsf,fd->bsd", h, w2)
        return out

    x = A_x
    xn = _layernorm(x, axis=-1)
    return x + _A_ref(xn, A_wq, A_wk, A_wv, A_wo) + _B_ref(xn, B_w1, B_w2)
```

```python
import functools
import math

import jax
import jax.numpy as jnp
from jax.experimental import pallas as pl
from jax.experimental.pallas import tpu as pltpu

_H = 32
_EPS = 1e-5
_TQ = 512
_KC = 128
_FC = 256

_NT = (((1,), (1,)), ((), ()))
_TN = (((0,), (0,)), ((), ()))


def _kernel(x_ref, wqt_ref, wk_ref, wvt_ref, wo_ref, w1_ref, w2_ref, o_ref,
            xn_ref, k_ref, vt_ref, qt_ref, ot_ref, sa_ref, sb_ref, *, seq, dh):
    f32, bf16 = jnp.float32, jnp.bfloat16
    tq, kc = _TQ, _KC
    nc = seq // kc
    i = pl.program_id(0)

    @pl.when(i == 0)
    def _():
        for r in range(0, seq, tq):
            x = x_ref[r:r + tq, :].astype(f32)
            mu = jnp.mean(x, axis=-1, keepdims=True)
            xc = x - mu
            var = jnp.mean(xc * xc, axis=-1, keepdims=True)
            xn = (xc * jax.lax.rsqrt(var + _EPS)).astype(bf16)
            xn_ref[r:r + tq, :] = xn
            k_ref[r:r + tq, :] = jnp.dot(
                xn, wk_ref[...], preferred_element_type=f32).astype(bf16)
            vt_ref[:, r:r + tq] = jax.lax.dot_general(
                wvt_ref[...], xn, _NT, preferred_element_type=f32).astype(bf16)

    row0 = pl.multiple_of(i * tq, tq)
    xn = xn_ref[pl.ds(row0, tq), :]

    scale = (dh ** -0.5) * math.log2(math.e)
    qt_ref[...] = (jax.lax.dot_general(
        wqt_ref[...], xn, _NT, preferred_element_type=f32) * scale).astype(bf16)

    def fused(h1, s_w, h2, s_r, m_r):
        if h1 is not None:
            q = qt_ref[pl.ds(pl.multiple_of(h1 * dh, dh), dh), :]
            m8 = jnp.full((8, tq), -jnp.inf, f32)
        if h2 is not None:
            l8 = jnp.zeros((8, tq), f32)
            o = jnp.zeros((dh, tq), f32)
        for c in range(nc):
            ks = slice(c * kc, (c + 1) * kc)
            if h1 is not None:
                s = jnp.dot(k_ref[ks, :], q, preferred_element_type=f32)
                s_w[ks, :] = s
                m8 = jnp.maximum(m8, jnp.max(s.reshape(kc // 8, 8, tq), axis=0))
            if h2 is not None:
                p = jnp.exp2(s_r[ks, :] - m_r)
                l8 = l8 + jnp.sum(p.reshape(kc // 8, 8, tq), axis=0)
                o = o + jnp.dot(vt_ref[:, ks], p.astype(bf16),
                                preferred_element_type=f32)
        if h2 is not None:
            l = jnp.sum(l8, axis=0, keepdims=True)
            ot_ref[pl.ds(pl.multiple_of(h2 * dh, dh), dh), :] = (o / l).astype(bf16)
        if h1 is not None:
            return jnp.max(m8, axis=0, keepdims=True)

    m0 = fused(0, sa_ref, None, None, None)

    def body(j, ma):
        mb = fused(2 * j + 1, sb_ref, 2 * j, sa_ref, ma)
        return fused(2 * j + 2, sa_ref, 2 * j + 1, sb_ref, mb)

    ma = jax.lax.fori_loop(0, _H // 2 - 1, body, m0)
    mb = fused(_H - 1, sb_ref, _H - 2, sa_ref, ma)
    fused(None, None, _H - 1, sb_ref, mb)

    acc = x_ref[pl.ds(row0, tq), :].astype(f32)
    acc = acc + jax.lax.dot_general(
        ot_ref[...], wo_ref[...], _TN, preferred_element_type=f32)
    ff = w1_ref.shape[1]
    for f0 in range(0, ff, _FC):
        h = jnp.dot(xn, w1_ref[:, f0:f0 + _FC], preferred_element_type=f32)
        h = h * jax.nn.sigmoid(h)
        acc = acc + jnp.dot(h.astype(bf16), w2_ref[f0:f0 + _FC, :],
                            preferred_element_type=f32)
    o_ref[...] = acc.astype(o_ref.dtype)


@jax.jit
def pallas_parallel_sum__grouped_kv_mqa__dense_activation_silu__prompt_kernel(
    A_x: jax.Array,
    A_wq: jax.Array,
    A_wk: jax.Array,
    A_wv: jax.Array,
    A_wo: jax.Array,
    B_x: jax.Array,
    B_w1: jax.Array,
    B_w2: jax.Array,
):
    del B_x
    b, seq, d = A_x.shape
    assert b == 1
    dh = A_wk.shape[1]
    ff = B_w1.shape[1]
    assert A_wq.shape == (d, _H * dh) and seq % _TQ == 0 and ff % _FC == 0
    bf16, f32 = jnp.bfloat16, jnp.float32

    def full(shape):
        return pl.BlockSpec(shape, lambda i: (0,) * len(shape))

    out = pl.pallas_call(
        functools.partial(_kernel, seq=seq, dh=dh),
        grid=(seq // _TQ,),
        in_specs=[
            full((seq, d)),
            full((_H * dh, d)),
            full((d, dh)),
            full((dh, d)),
            full((_H * dh, d)),
            full((d, ff)),
            full((ff, d)),
        ],
        out_specs=pl.BlockSpec((_TQ, d), lambda i: (i, 0)),
        out_shape=jax.ShapeDtypeStruct((seq, d), A_x.dtype),
        scratch_shapes=[
            pltpu.VMEM((seq, d), bf16),
            pltpu.VMEM((seq, dh), bf16),
            pltpu.VMEM((dh, seq), bf16),
            pltpu.VMEM((_H * dh, _TQ), bf16),
            pltpu.VMEM((_H * dh, _TQ), bf16),
            pltpu.VMEM((seq, _TQ), f32),
            pltpu.VMEM((seq, _TQ), f32),
        ],
        compiler_params=pltpu.CompilerParams(
            dimension_semantics=("arbitrary",),
            vmem_limit_bytes=100 * 1024 * 1024,
        ),
    )(A_x.reshape(seq, d), A_wq.T, A_wk, A_wv.T, A_wo, B_w1, B_w2)
    return out.reshape(b, seq, d)
```

```python
import functools
import math

import jax
import jax.numpy as jnp
from jax.experimental import pallas as pl
from jax.experimental.pallas import tpu as pltpu

_H = 32
_EPS = 1e-5
_TQ = 512
_KC = 128
_U = 2
_FC = 256
_FR = 128
_XSPLIT = (0, 256, 768)
_LNEDGES = (0,)
_LNR = 256

_NT = (((1,), (1,)), ((), ()))
_TN = (((0,), (0,)), ((), ()))


def _kernel(x_hbm, wq_ref, wkt_ref, wvt_ref, wo_hbm, w1_hbm, w2_hbm, o_ref,
            x_ref, wo_ref, w1_ref, w2_ref, sems, wqkvt_ref,
            xn_ref, k_ref, vt_ref, qt_ref, ot_ref, acc_ref, m_ref, *s_refs,
            seq, dh):
    f32, bf16 = jnp.float32, jnp.bfloat16
    tq, kc, U = _TQ, _KC, _U
    nc = seq // kc
    nq = seq // tq
    nb = _H // U
    hd = _H * dh
    ff = w1_ref.shape[1]
    i = pl.program_id(0)
    row0 = pl.multiple_of(i * tq, tq)

    xb = list(_XSPLIT) + [seq]
    x_copies = [
        pltpu.make_async_copy(x_hbm.at[a:b], x_ref.at[a:b], sems.at[n])
        for n, (a, b) in enumerate(zip(xb[:-1], xb[1:]))]
    w_copies = [
        pltpu.make_async_copy(src, dst, sems.at[len(_XSPLIT) + n])
        for n, (src, dst) in enumerate(
            [(w1_hbm, w1_ref), (w2_hbm, w2_ref), (wo_hbm, wo_ref)])]

    def fused(q1, h1, s_w, h2, s_r, m_r, filler=None):
        if h1 is not None:
            q = qt_ref[q1, pl.ds(pl.multiple_of(h1 * dh, dh), dh), :]
            m8 = jnp.full((8, tq), -jnp.inf, f32)
        if h2 is not None:
            l8 = jnp.zeros((8, tq), f32)
            o = jnp.zeros((dh, tq), f32)
        for c in range(nc):
            ks = slice(c * kc, (c + 1) * kc)
            if filler is not None:
                filler()
            if h1 is not None:
                s = jnp.dot(k_ref[ks, :], q, preferred_element_type=f32)
                s_w[ks, :] = s
                m8 = jnp.maximum(m8, jnp.max(s.reshape(kc // 8, 8, tq), axis=0))
            if h2 is not None:
                p = jnp.exp2(s_r[ks, :] - m_r)
                p3 = p.reshape(kc // 8, 8, tq)
                for g in reversed(range(kc // 8)):
                    l8 = l8 + p3[g]
                o = o + jnp.dot(vt_ref[:, ks], p.astype(bf16),
                                preferred_element_type=f32)
        if h2 is not None:
            l = jnp.sum(l8, axis=0, keepdims=True)
            ot_ref[pl.ds(pl.multiple_of(h2 * dh, dh), dh), :] = (o / l).astype(bf16)
        if h1 is not None:
            return jnp.max(m8, axis=0, keepdims=True)

    def block(qw, jw, pw, jr, pr, filler=None):
        ms = None if jr is None else [m_ref[pr * U + u] for u in range(U)]
        for u in range(U):
            hw = None if jw is None else jw * U + u
            hr = None if jr is None else jr * U + u
            sw = None if jw is None else s_refs[pw * U + u]
            sr = None if jr is None else s_refs[pr * U + u]
            m = fused(qw, hw, sw, hr, sr, None if jr is None else ms[u], filler)
            if jw is not None:
                m_ref[pw * U + u] = m

    @pl.when(i == 0)
    def _():
        scale = (dh ** -0.5) * math.log2(math.e)
        for cp in x_copies:
            cp.start()
        for cp in w_copies:
            cp.start()
        wqkvt_ref[0:hd, :] = wq_ref[...].T
        wqkvt_ref[hd:hd + dh, :] = wkt_ref[...]
        wqkvt_ref[hd + dh:, :] = wvt_ref[...]

        def layernorm(a, b):
            if a in _XSPLIT:
                x_copies[_XSPLIT.index(a)].wait()
            x = x_ref[a:b, :].astype(f32)
            mu = jnp.mean(x, axis=-1, keepdims=True)
            xc = x - mu
            var = jnp.mean(xc * xc, axis=-1, keepdims=True)
            xn_ref[a:b, :] = (xc * jax.lax.rsqrt(var + _EPS)).astype(bf16)

        def project(a, b):
            qkv = jax.lax.dot_general(
                wqkvt_ref[...], xn_ref[a:b, :], _NT, preferred_element_type=f32)
            qt_ref[a // tq, :, a % tq:a % tq + b - a] = (qkv[:hd] * scale).astype(bf16)
            k_ref[a:b, :] = qkv[hd:hd + dh].T.astype(bf16)
            vt_ref[:, a:b] = qkv[hd + dh:].astype(bf16)

        edges = list(_LNEDGES) + list(range(_LNEDGES[-1] + _LNR, seq + 1, _LNR))
        spans = list(zip(edges[:-1], edges[1:]))
        layernorm(*spans[0])
        for n, span in enumerate(spans):
            if n + 1 < len(spans):
                layernorm(*spans[n + 1])
            project(*span)
        block(0, 0, 0, None, None)

    def body(j, carry):
        wrap = (j + 1) // nb
        qw = i + wrap
        jw = (j + 1) - wrap * nb

        @pl.when(j % 2 == 0)
        def _():
            block(qw, jw, 1, j, 0)

        @pl.when(j % 2 == 1)
        def _():
            block(qw, jw, 0, j, 1)

        return carry

    last = i == nq - 1
    jax.lax.fori_loop(0, jnp.where(last, nb - 1, nb), body, 0)

    @pl.when(i == 0)
    def _():
        for cp in w_copies:
            cp.wait()

    def ffn_pieces(fr):
        items = [(r, f0) for r in range(0, tq, fr) for f0 in range(0, ff, _FC)]

        def mm1(r, f0):
            rows = pl.ds(pl.multiple_of(row0 + r, fr), fr)
            return jnp.dot(xn_ref[rows, :], w1_ref[:, f0:f0 + _FC],
                           preferred_element_type=f32)

        h_next = mm1(*items[0])
        yield
        acc = None
        for n, (r, f0) in enumerate(items):
            h = h_next
            if n + 1 < len(items):
                h_next = mm1(*items[n + 1])
                yield
            if f0 == 0:
                rows = pl.ds(pl.multiple_of(row0 + r, fr), fr)
                acc = x_ref[rows, :].astype(f32)
            h = h * jax.nn.sigmoid(h)
            acc = acc + jnp.dot(h.astype(bf16), w2_ref[f0:f0 + _FC, :],
                                preferred_element_type=f32)
            if f0 + _FC == ff:
                acc_ref[r:r + fr, :] = acc
            yield

    def finish():
        o_ref[...] = (acc_ref[...] + jax.lax.dot_general(
            ot_ref[...], wo_ref[...], _TN,
            preferred_element_type=f32)).astype(o_ref.dtype)

    @pl.when(jnp.logical_not(last))
    def _():
        for _ in ffn_pieces(tq):
            pass
        finish()

    @pl.when(last)
    def _():
        gen = ffn_pieces(_FR)
        block(None, None, None, nb - 1, (nb - 1) % 2,
              filler=lambda: next(gen, None))
        for _ in gen:
            pass
        finish()


@jax.jit
def pallas_parallel_sum__grouped_kv_mqa__dense_activation_silu__prompt_kernel(
    A_x: jax.Array,
    A_wq: jax.Array,
    A_wk: jax.Array,
    A_wv: jax.Array,
    A_wo: jax.Array,
    B_x: jax.Array,
    B_w1: jax.Array,
    B_w2: jax.Array,
):
    del B_x
    b, seq, d = A_x.shape
    assert b == 1
    dh = A_wk.shape[1]
    ff = B_w1.shape[1]
    hd = _H * dh
    assert A_wq.shape == (d, hd) and seq % _TQ == 0 and ff % _FC == 0
    assert (_H // _U) % 2 == 0
    bf16, f32 = jnp.bfloat16, jnp.float32

    def full(shape):
        return pl.BlockSpec(shape, lambda i: (0,) * len(shape))

    hbm = pl.BlockSpec(memory_space=pl.ANY)

    out = pl.pallas_call(
        functools.partial(_kernel, seq=seq, dh=dh),
        grid=(seq // _TQ,),
        in_specs=[
            hbm,
            full((d, hd)),
            full((dh, d)),
            full((dh, d)),
            hbm,
            hbm,
            hbm,
        ],
        out_specs=pl.BlockSpec((_TQ, d), lambda i: (i, 0)),
        out_shape=jax.ShapeDtypeStruct((seq, d), A_x.dtype),
        scratch_shapes=[
            pltpu.VMEM((seq, d), bf16),
            pltpu.VMEM((hd, d), bf16),
            pltpu.VMEM((d, ff), bf16),
            pltpu.VMEM((ff, d), bf16),
            pltpu.SemaphoreType.DMA((len(_XSPLIT) + 3,)),
            pltpu.VMEM((hd + 2 * dh, d), bf16),
            pltpu.VMEM((seq, d), bf16),
            pltpu.VMEM((seq, dh), bf16),
            pltpu.VMEM((dh, seq), bf16),
            pltpu.VMEM((seq // _TQ, hd, _TQ), bf16),
            pltpu.VMEM((hd, _TQ), bf16),
            pltpu.VMEM((_TQ, d), f32),
            pltpu.VMEM((2 * _U, 1, _TQ), f32),
        ] + [pltpu.VMEM((seq, _TQ), f32)] * (2 * _U),
        compiler_params=pltpu.CompilerParams(
            dimension_semantics=("arbitrary",),
            vmem_limit_bytes=110 * 1024 * 1024,
        ),
    )(A_x.reshape(seq, d), A_wq, A_wk.T, A_wv.T, A_wo, B_w1, B_w2)
    return out.reshape(b, seq, d)
```

```python
import functools
import math

import jax
import jax.numpy as jnp
from jax.experimental import pallas as pl
from jax.experimental.pallas import tpu as pltpu

_H = 32
_EPS = 1e-5
_TQ = 512
_KC = 128
_U = 2
_G = 12
_PW = 128
_PFRAC = 1.0
_ZL = 0
_FC = 256
_FR = 128
_XSPLIT = (0, 256, 768)
_LNEDGES = (0,)
_LNR = 256

_NT = (((1,), (1,)), ((), ()))
_TN = (((0,), (0,)), ((), ()))


def _kernel(x_hbm, wq_ref, wkt_ref, wvt_ref, wo_hbm, w1_hbm, w2_hbm, o_ref,
            x_ref, wo_ref, w1_ref, w2_ref, sems, wqkvt_ref,
            xn_ref, k_ref, vt_ref, qt_ref, ot_ref, acc_ref, m_ref, kb_ref, z_ref,
            *rest, seq, dh):
    qf_refs, s_refs = rest[:_U], rest[_U:]
    f32, bf16 = jnp.float32, jnp.bfloat16
    tq, kc, U = _TQ, _KC, _U
    nc = seq // kc
    nq = seq // tq
    nb = _H // U
    hd = _H * dh
    ff = w1_ref.shape[1]
    i = pl.program_id(0)
    row0 = pl.multiple_of(i * tq, tq)

    xb = list(_XSPLIT) + [seq]
    x_copies = [
        pltpu.make_async_copy(x_hbm.at[a:b], x_ref.at[a:b], sems.at[n])
        for n, (a, b) in enumerate(zip(xb[:-1], xb[1:]))]
    w_copies = [
        pltpu.make_async_copy(src, dst, sems.at[len(_XSPLIT) + n])
        for n, (src, dst) in enumerate(
            [(w1_hbm, w1_ref), (w2_hbm, w2_ref), (wo_hbm, wo_ref)])]

    nv = _G * 16
    nm = seq - nv
    nw = tq // _PW
    vpos = {}
    for w in range(nw):
        for j in range(nv // 8):
            g = int((j + w / nw) * (nm // 8) * _PFRAC / (nv // 8))
            vpos.setdefault((w, g), []).append(j)

    medges = [16 * ((c * (nm // 16) + nc - 1) // nc) for c in range(nc + 1)]

    def fused(q, s_w, qf_ref, s_r, m_r, filler=None):
        m = ot = None
        if q is not None:
            m8 = [jnp.full((8, _PW), -jnp.inf, f32)] * nw
        if s_r is not None:
            l8 = z_ref[0:8, :] if _ZL else jnp.zeros((8, tq), f32)
            o = z_ref[...]
        for c in range(nc):
            ks = slice(c * kc, (c + 1) * kc)
            if filler is not None:
                filler()
            if q is not None:
                a, b = medges[c], medges[c + 1]
                s = jnp.dot(k_ref[a:b, :], q, preferred_element_type=f32)
                s_w[a:b, :] = s
                for g in range(a // 8, b // 8):
                    for w in range(nw):
                        cs = slice(w * _PW, (w + 1) * _PW)
                        for j in vpos.get((w, g), ()):
                            sv = None
                            for d in range(dh):
                                kb = kb_ref[d, j * 8:(j + 1) * 8, :]
                                if _PW > 128:
                                    kb = jnp.concatenate([kb] * (_PW // 128), axis=1)
                                t = kb * qf_ref[d:d + 1, cs]
                                sv = t if d == 0 else sv + t
                            s_w[nm + j * 8:nm + (j + 1) * 8, cs] = sv
                            m8[w] = jnp.maximum(m8[w], sv)
                        m8[w] = jnp.maximum(
                            m8[w], s[g * 8 - a:(g + 1) * 8 - a, cs])
            if s_r is not None:
                p = jnp.exp2(s_r[ks, :] - m_r)
                p3 = p.reshape(kc // 8, 8, tq)
                for g in reversed(range(kc // 8)):
                    l8 = l8 + p3[g]
                o = o + jnp.dot(vt_ref[:, ks], p.astype(bf16),
                                preferred_element_type=f32)
        if s_r is not None:
            ot = (o / jnp.sum(l8, axis=0, keepdims=True)).astype(bf16)
        if q is not None:
            m = jnp.max(jnp.concatenate(m8, axis=1), axis=0, keepdims=True)
        return m, ot

    def block(qw, jw, pw, jr, pr, filler=None):
        qs = ms = [None] * U
        if jw is not None:
            qall = qt_ref[qw, pl.ds(pl.multiple_of(jw * (U * dh), U * dh), U * dh), :]
            qs = [qall[u * dh:(u + 1) * dh] for u in range(U)]
            if nv:
                for u in range(U):
                    qf_refs[u][...] = qs[u].astype(f32)
        if jr is not None:
            ms = [m_ref[pr * U + u] for u in range(U)]
        res = [fused(qs[u], None if jw is None else s_refs[pw * U + u], qf_refs[u],
                     None if jr is None else s_refs[pr * U + u], ms[u], filler)
               for u in range(U)]
        if jw is not None:
            for u in range(U):
                m_ref[pw * U + u] = res[u][0]
        if jr is not None:
            ot_ref[pl.ds(pl.multiple_of(jr * (U * dh), U * dh), U * dh), :] = (
                jnp.concatenate([r[1] for r in res], axis=0))

    @pl.when(i == 0)
    def _():
        scale = (dh ** -0.5) * math.log2(math.e)
        for cp in x_copies:
            cp.start()
        for cp in w_copies:
            cp.start()
        z_ref[...] = jnp.zeros(z_ref.shape, f32)
        wqkvt_ref[0:hd, :] = wq_ref[...].T
        wqkvt_ref[hd:hd + dh, :] = wkt_ref[...]
        wqkvt_ref[hd + dh:, :] = wvt_ref[...]

        def layernorm(a, b):
            if a in _XSPLIT:
                x_copies[_XSPLIT.index(a)].wait()
            x = x_ref[a:b, :].astype(f32)
            mu = jnp.mean(x, axis=-1, keepdims=True)
            xc = x - mu
            var = jnp.mean(xc * xc, axis=-1, keepdims=True)
            xn_ref[a:b, :] = (xc * jax.lax.rsqrt(var + _EPS)).astype(bf16)

        def project(a, b):
            qkv = jax.lax.dot_general(
                wqkvt_ref[...], xn_ref[a:b, :], _NT, preferred_element_type=f32)
            qt_ref[a // tq, :, a % tq:a % tq + b - a] = (qkv[:hd] * scale).astype(bf16)
            k_ref[a:b, :] = qkv[hd:hd + dh].T.astype(bf16)
            vt_ref[:, a:b] = qkv[hd + dh:].astype(bf16)

        edges = list(_LNEDGES) + list(range(_LNEDGES[-1] + _LNR, seq + 1, _LNR))
        spans = list(zip(edges[:-1], edges[1:]))
        layernorm(*spans[0])
        for n, span in enumerate(spans):
            if n + 1 < len(spans):
                layernorm(*spans[n + 1])
            project(*span)
        if nv:
            kv = k_ref[nm:, :].astype(f32)
            for d in range(dh):
                kb_ref[d] = jnp.broadcast_to(kv[:, d:d + 1], (nv, 128))
        block(0, 0, 0, None, None)

    def body(j, carry):
        wrap = (j + 1) // nb
        qw = i + wrap
        jw = (j + 1) - wrap * nb

        @pl.when(j % 2 == 0)
        def _():
            block(qw, jw, 1, j, 0)

        @pl.when(j % 2 == 1)
        def _():
            block(qw, jw, 0, j, 1)

        return carry

    last = i == nq - 1
    jax.lax.fori_loop(0, jnp.where(last, nb - 1, nb), body, 0)

    @pl.when(i == 0)
    def _():
        for cp in w_copies:
            cp.wait()

    def ffn_pieces(fr):
        items = [(r, f0) for r in range(0, tq, fr) for f0 in range(0, ff, _FC)]

        def mm1(r, f0):
            rows = pl.ds(pl.multiple_of(row0 + r, fr), fr)
            return jnp.dot(xn_ref[rows, :], w1_ref[:, f0:f0 + _FC],
                           preferred_element_type=f32)

        h_next = mm1(*items[0])
        yield
        acc = None
        for n, (r, f0) in enumerate(items):
            h = h_next
            if n + 1 < len(items):
                h_next = mm1(*items[n + 1])
                yield
            if f0 == 0:
                rows = pl.ds(pl.multiple_of(row0 + r, fr), fr)
                acc = x_ref[rows, :].astype(f32)
            h = h * jax.nn.sigmoid(h)
            acc = acc + jnp.dot(h.astype(bf16), w2_ref[f0:f0 + _FC, :],
                                preferred_element_type=f32)
            if f0 + _FC == ff:
                acc_ref[r:r + fr, :] = acc
            yield

    def finish():
        o_ref[...] = (acc_ref[...] + jax.lax.dot_general(
            ot_ref[...], wo_ref[...], _TN,
            preferred_element_type=f32)).astype(o_ref.dtype)

    @pl.when(jnp.logical_not(last))
    def _():
        for _ in ffn_pieces(tq):
            pass
        finish()

    @pl.when(last)
    def _():
        gen = ffn_pieces(_FR)
        block(None, None, None, nb - 1, (nb - 1) % 2,
              filler=lambda: next(gen, None))
        for _ in gen:
            pass
        finish()


@jax.jit
def pallas_parallel_sum__grouped_kv_mqa__dense_activation_silu__prompt_kernel(
    A_x: jax.Array,
    A_wq: jax.Array,
    A_wk: jax.Array,
    A_wv: jax.Array,
    A_wo: jax.Array,
    B_x: jax.Array,
    B_w1: jax.Array,
    B_w2: jax.Array,
):
    del B_x
    b, seq, d = A_x.shape
    assert b == 1
    dh = A_wk.shape[1]
    ff = B_w1.shape[1]
    hd = _H * dh
    assert A_wq.shape == (d, hd) and seq % _TQ == 0 and ff % _FC == 0
    assert (_H // _U) % 2 == 0
    bf16, f32 = jnp.bfloat16, jnp.float32

    def full(shape):
        return pl.BlockSpec(shape, lambda i: (0,) * len(shape))

    hbm = pl.BlockSpec(memory_space=pl.ANY)

    out = pl.pallas_call(
        functools.partial(_kernel, seq=seq, dh=dh),
        grid=(seq // _TQ,),
        in_specs=[
            hbm,
            full((d, hd)),
            full((dh, d)),
            full((dh, d)),
            hbm,
            hbm,
            hbm,
        ],
        out_specs=pl.BlockSpec((_TQ, d), lambda i: (i, 0)),
        out_shape=jax.ShapeDtypeStruct((seq, d), A_x.dtype),
        scratch_shapes=[
            pltpu.VMEM((seq, d), bf16),
            pltpu.VMEM((hd, d), bf16),
            pltpu.VMEM((d, ff), bf16),
            pltpu.VMEM((ff, d), bf16),
            pltpu.SemaphoreType.DMA((len(_XSPLIT) + 3,)),
            pltpu.VMEM((hd + 2 * dh, d), bf16),
            pltpu.VMEM((seq, d), bf16),
            pltpu.VMEM((seq, dh), bf16),
            pltpu.VMEM((dh, seq), bf16),
            pltpu.VMEM((seq // _TQ, hd, _TQ), bf16),
            pltpu.VMEM((hd, _TQ), bf16),
            pltpu.VMEM((_TQ, d), f32),
            pltpu.VMEM((2 * _U, 1, _TQ), f32),
            pltpu.VMEM((dh, max(_G * 16, 8), 128), f32),
            pltpu.VMEM((dh, _TQ), f32),
        ] + [pltpu.VMEM((dh, _TQ), f32)] * _U
        + [pltpu.VMEM((seq, _TQ), f32)] * (2 * _U),
        compiler_params=pltpu.CompilerParams(
            dimension_semantics=("arbitrary",),
            vmem_limit_bytes=110 * 1024 * 1024,
        ),
    )(A_x.reshape(seq, d), A_wq, A_wk.T, A_wv.T, A_wo, B_w1, B_w2)
    return out.reshape(b, seq, d)
```

```python
import functools
import math

import jax
import jax.numpy as jnp
from jax.experimental import pallas as pl
from jax.experimental.pallas import tpu as pltpu

_H = 32
_EPS = 1e-5
_TQ = 512
_KC = 128
_U = 16
_G = 17
_CUMA = 0
_FEND = 1
_DELTA = -2
_PH = 2
_FW = 8
_NFB = 1
_FT = 1.0
_NQF = 4
_NKB = 1
_LEAD = 10
_SC = 256
_L_MIN, _L_MAX = 2.0 ** -40, 2.0 ** 64
_V_MIN, _V_MAX = 2.0 ** -30, 2.0 ** 60
_FC = 256
_XSPLIT = (0, 256, 512, 1024)
_WLATE = 1
_KLAG = 1
_W1 = 1
_NEARLY = 1
_LNR = 256

_NT = (((1,), (1,)), ((), ()))
_TN = (((0,), (0,)), ((), ()))


def _plan(nc, nw, nffn, fslots):
    ng = _KC // 16
    cum = [int(_G * (c + _CUMA) / (nc - 1 + _CUMA)) if c else 0 for c in range(nc)]
    vg = [[7, 6, 5, 4][:cum[c] - cum[c - 1]] if c else [] for c in range(nc)]
    seqn = [(u, c) for u in range(_U) for c in range(nc)]
    stream, ends = [], []
    for u, c in seqn:
        stream += [(u, c, g) for g in reversed(range(ng)) if g not in vg[c]]
        ends.append(len(stream))
    npv = len(seqn)
    fpos = [npv - _FEND] * nffn
    events, when = [], {}
    now = issued = nf = lt = 0
    lwhen = {}
    for t, (u, c) in enumerate(seqn):
        extra = _FW * sum(1 for f in fpos if f == t)
        batch = []
        while issued < len(stream) and (
                issued < ends[t]
                or lt + extra - lwhen[stream[ends[t] - 1]] < _LEAD):
            when[stream[issued]] = now
            lwhen[stream[issued]] = lt
            batch.append(stream[issued])
            issued += 1
            now += 1
            lt += 1
        if batch:
            events.append(("s", batch))
        while nf < nffn and fpos[nf] == t:
            events.append(("ffn", nf))
            nf += 1
            now += fslots * _FT
            lt += _FW
        events.append(("pv", u, c))
        now += 1
        lt += 1
    pieces = [(c, 2 * g + e) for c in range(nc) for g in vg[c] for e in (1, 0)]
    at = {}
    for u in range(_U):
        chain = []
        for c in range(nc):
            mg = [g for g in reversed(range(ng)) if g not in vg[c]]
            chain += [(when[(u, c, g)] + 0.5 * e, c, 2 * n + e)
                      for n, g in enumerate(mg) for e in (0, 1)]
        last = {c: max(k for k, it in enumerate(chain) if it[1] == c)
                for c in range(nc)}
        t0 = chain[0][0] - (_DELTA if u else 0)
        t1 = chain[last[nc - 2]][0]
        for w in range(nw):
            for n, (c, r) in enumerate(pieces):
                tt = t0 + (n + (w + _PH) / nw) * (t1 - t0) / len(pieces)
                k = min(k for k, it in enumerate(chain) if it[0] >= tt)
                k = min(k, last[c - 1])
                at.setdefault((u, chain[k][1], chain[k][2], w), []).append((c, r))
    return vg, events, at


def _kernel(x_hbm, wq_hbm, wkt_hbm, wvt_hbm, wo_hbm, w1_hbm, w2_hbm, o_ref,
            x_ref, wq_ref, wo_ref, w1_ref, w2_ref, sems, wqkvt_ref, kt_ref,
            xn_ref, k_ref, vt_ref, qt_ref, ot_ref, kb_ref, z_ref, vok_ref, s_ref, h_ref, acc_ref,
            *rest, seq, dh):
    qf_refs, pv_refs = rest[:_U], rest[_U:]
    f32, bf16 = jnp.float32, jnp.bfloat16
    tq, kc, U = _TQ, _KC, _U
    nc = seq // kc
    nb = _H // U
    hd = _H * dh
    ff = w1_ref.shape[1]
    nw = tq // 128
    i = pl.program_id(0)
    row0 = pl.multiple_of(i * tq, tq)

    xb = list(_XSPLIT) + [seq]
    x_copies = [
        pltpu.make_async_copy(x_hbm.at[a:b], x_ref.at[a:b], sems.at[n])
        for n, (a, b) in enumerate(zip(xb[:-1], xb[1:]))]
    w_copies = [
        pltpu.make_async_copy(src, dst, sems.at[len(_XSPLIT) + n])
        for n, (src, dst) in enumerate(
            [(w1_hbm, w1_ref), (w2_hbm, w2_ref), (wo_hbm, wo_ref)])]

    wq_copies = [
        pltpu.make_async_copy(src, dst, sems.at[len(_XSPLIT) + 3 + n])
        for n, (src, dst) in enumerate(
            [(wq_hbm, wq_ref), (wkt_hbm, wqkvt_ref.at[0:dh]),
             (wvt_hbm, wqkvt_ref.at[dh:2 * dh])])]

    fr = tq // nb
    nf = ff // 128
    vg, events, at = _plan(nc, nw, _NFB, fr // 16)
    vslot = {}
    for c in range(nc):
        for g in vg[c]:
            vslot[(c, g)] = len(vslot)

    def silu2(h):
        return (h + h * jnp.tanh(h)).astype(bf16)

    def heads_fast(qs, frows, arows):
        nh = len(qs)
        l8 = [[jnp.zeros((8, 128), f32)] * nw for _ in range(nh)]
        o = [z_ref[...] for _ in range(nh)]
        pms = {}
        outs, oks = [], []

        def vpu_piece(u, c, r, w):
            slot = vslot[(c, r // 2)] * 2 + r % 2
            sv = None
            for d in range(dh):
                t = (kb_ref[w * _NKB // nw, d, slot * 8:(slot + 1) * 8, :]
                     * qf_refs[u][slot % _NQF, d:d + 1, w * 128:(w + 1) * 128])
                sv = t if d == 0 else sv + t
            p = jnp.exp2(sv)
            pv_refs[u][slot * 8:(slot + 1) * 8, w * 128:(w + 1) * 128] = p
            l8[u][w] = l8[u][w] + p

        def scores(items):
            for u in sorted(set(it[0] for it in items)):
                its = [it for it in items if it[0] == u]
                lhs = pltpu.bitcast(jnp.concatenate(
                    [k_ref[c * kc // 2 + g * 8:c * kc // 2 + (g + 1) * 8, :]
                     for _, c, g in its], axis=0), bf16)
                pm = jnp.exp2(jnp.dot(lhs, qs[u], preferred_element_type=f32))
                for n, it in enumerate(its):
                    pms[it] = pm[n * 16:(n + 1) * 16, :]

        def pv_mm(u, c):
            mg = [g for g in range(kc // 16) if g not in vg[c]]
            tiles = {}
            pos = 0
            for g in mg[::-1]:
                pm = pms.pop((u, c, g))
                for e in (0, 1):
                    row = pm[e * 8:e * 8 + 8, :]
                    tiles[2 * g + e] = row
                    for w in range(nw):
                        for cc, r in at.get((u, c, pos, w), ()):
                            vpu_piece(u, cc, r, w)
                        l8[u][w] = l8[u][w] + row[:, w * 128:(w + 1) * 128]
                    pos += 1
            for g in vg[c]:
                for e in (0, 1):
                    slot = vslot[(c, g)] * 2 + e
                    tiles[2 * g + e] = pv_refs[u][slot * 8:(slot + 1) * 8, :]
            p = jnp.concatenate([tiles[r] for r in range(kc // 8)], axis=0)
            o[u] = o[u] + jnp.dot(
                pltpu.bitcast(vt_ref[:, c * kc:(c + 1) * kc], bf16),
                p.astype(bf16), preferred_element_type=f32)
            if c == nc - 1:
                l = jnp.sum(jnp.concatenate(l8[u], axis=1), axis=0, keepdims=True)
                outs.append((o[u] / l).astype(bf16))
                oks.append(jnp.logical_and(l >= _L_MIN, l <= _L_MAX))

        def ffn_mm(k):
            fs = slice(k * 128, (k + 1) * 128)
            h_ref[arows, fs] = silu2(0.5 * jnp.dot(
                xn_ref[frows, :], w1_ref[:, fs], preferred_element_type=f32))

        for ev in events:
            if ev[0] == "s":
                scores(ev[1])
            elif ev[0] == "pv":
                pv_mm(ev[1], ev[2])
            else:
                ffn_mm(ev[1])
        ok = functools.reduce(jnp.logical_and, oks)
        return jnp.concatenate(outs, axis=0), jnp.where(ok, 1.0, 0.0)

    @pl.when(i == 0)
    def _():
        scale = (dh ** -0.5) * math.log2(math.e)
        x_copies[0].start()
        for cp in wq_copies:
            cp.start()
        for cp in x_copies[1:_NEARLY]:
            cp.start()
        if not _WLATE:
            for cp in w_copies:
                cp.start()
        z_ref[...] = jnp.zeros(z_ref.shape, f32)

        def layernorm(a, b):
            if a in _XSPLIT and not (_W1 and a == _LNR):
                x_copies[_XSPLIT.index(a)].wait()
                if a == 0:
                    for cp in x_copies[_NEARLY:]:
                        cp.start()
                if _WLATE and a == _XSPLIT[-1]:
                    for cp in w_copies:
                        cp.start()
            x = x_ref[a:b, :].astype(f32)
            mu = jnp.mean(x, axis=-1, keepdims=True)
            xc = x - mu
            var = jnp.mean(xc * xc, axis=-1, keepdims=True)
            xn_ref[a:b, :] = (xc * jax.lax.rsqrt(var + _EPS)).astype(bf16)

        def project(a, b):
            qkv = jax.lax.dot_general(
                wqkvt_ref[...], xn_ref[a:b, :], _NT, preferred_element_type=f32)
            kt_ref[:, a:b] = qkv[0:dh]
            vt_ref[:, a:b] = pltpu.bitcast(qkv[dh:2 * dh].astype(bf16), jnp.uint32)
            qt_ref[a // tq, :, a % tq:a % tq + b - a] = (
                qkv[2 * dh:] * scale).astype(bf16)

        def keys(a, b):
            k = kt_ref[:, a:b].T.astype(bf16)
            k_ref[a // 2:b // 2, :] = pltpu.bitcast(k, jnp.uint32)
            kf = k.astype(f32)
            for (c, g), slot in vslot.items():
                r0 = c * kc + g * 16
                if a <= r0 < b:
                    for d in range(dh):
                        kb = jnp.broadcast_to(
                            kf[r0 - a:r0 - a + 16, d:d + 1], (16, 128))
                        for n in range(_NKB):
                            kb_ref[n, d, slot * 16:(slot + 1) * 16, :] = kb

        edges = list(range(0, seq + 1, _LNR))
        spans = list(zip(edges[:-1], edges[1:]))
        layernorm(*spans[0])
        for cp in wq_copies:
            cp.wait()
        if _W1 and _LNR in _XSPLIT:
            x_copies[_XSPLIT.index(_LNR)].wait()
        wqkvt_ref[2 * dh:, :] = wq_ref[...].T
        done = 0
        for n, span in enumerate(spans):
            if n + 1 < len(spans):
                layernorm(*spans[n + 1])
            project(*span)
            while done <= n and (done + _KLAG <= n or span[1] > _XSPLIT[-1]):
                keys(*spans[done])
                done += 1
        vmax = jnp.max(jnp.abs(pltpu.bitcast(vt_ref[...], bf16).astype(f32)), keepdims=True)
        vok = jnp.logical_and(vmax >= _V_MIN, vmax <= _V_MAX)
        vok_ref[...] = jnp.broadcast_to(jnp.where(vok, 1.0, 0.0), vok_ref.shape)
        w_copies[0].wait()

    def body(j, carry):
        rows = pl.ds(pl.multiple_of(j * (U * dh), U * dh), U * dh)
        qall = qt_ref[i, rows, :]
        qs = [qall[u * dh:(u + 1) * dh] for u in range(U)]
        for u in range(U):
            qf = qs[u].astype(f32)
            for n in range(_NQF):
                qf_refs[u][n] = qf
        ot, ok = heads_fast(qs, pl.ds(pl.multiple_of(row0 + j * fr, fr), fr),
                            pl.ds(pl.multiple_of(j * fr, fr), fr))
        ot_ref[rows, :] = ot
        return jnp.minimum(carry, ok)

    ok = jax.lax.fori_loop(0, nb, body, vok_ref[...])

    @pl.when(i == 0)
    def _():
        w_copies[1].wait()
        w_copies[2].wait()

    rows = pl.ds(row0, tq)
    xn = xn_ref[rows, :]
    acc = x_ref[rows, :].astype(f32)
    f_lo = 128 * _NFB
    fedges = ([0] if _NFB else []) + list(range(f_lo, ff, _FC)) + [ff]
    fspans = list(zip(fedges[:-1], fedges[1:]))

    def hidden(a, b):
        if b <= f_lo:
            return h_ref[...]
        return silu2(0.5 * jnp.dot(xn, w1_ref[:, a:b], preferred_element_type=f32))

    h_next = hidden(*fspans[0])
    for n, (a, b) in enumerate(fspans):
        h = h_next
        if n + 1 < len(fspans):
            h_next = hidden(*fspans[n + 1])
        acc = acc + jnp.dot(h, w2_ref[a:b, :], preferred_element_type=f32)
    acc_ref[...] = acc
    o_ref[...] = (acc + jax.lax.dot_general(
        ot_ref[...], wo_ref[...], _TN,
        preferred_element_type=f32)).astype(o_ref.dtype)

    @pl.when(jnp.min(ok) < 0.5)
    def _():
        def safe_head(h, carry):
            rows = pl.ds(pl.multiple_of(h * dh, dh), dh)
            q = qt_ref[i, rows, :]

            def pass1(c, m8):
                kr = pl.ds(pl.multiple_of(c * (_SC // 2), _SC // 2), _SC // 2)
                s = jnp.dot(pltpu.bitcast(k_ref[kr, :], bf16), q,
                            preferred_element_type=f32)
                s_ref[pl.ds(pl.multiple_of(c * _SC, _SC), _SC), :] = s
                return jnp.maximum(
                    m8, jnp.max(s.reshape(_SC // 8, 8, tq), axis=0))

            m8 = jax.lax.fori_loop(0, seq // _SC, pass1,
                                   jnp.full((8, tq), -jnp.inf, f32))
            m = jnp.max(m8, axis=0, keepdims=True)

            def pass2(c, lo):
                ks = pl.ds(pl.multiple_of(c * _SC, _SC), _SC)
                p = jnp.exp2(s_ref[ks, :] - m)
                return (lo[0] + jnp.sum(p.reshape(_SC // 8, 8, tq), axis=0),
                        lo[1] + jnp.dot(pltpu.bitcast(vt_ref[:, ks], bf16),
                                        p.astype(bf16),
                                        preferred_element_type=f32))

            l8, o = jax.lax.fori_loop(
                0, seq // _SC, pass2,
                (jnp.zeros((8, tq), f32), jnp.zeros((dh, tq), f32)))
            l = jnp.sum(l8, axis=0, keepdims=True)
            ot_ref[rows, :] = (o / l).astype(bf16)
            return carry

        jax.lax.fori_loop(0, _H, safe_head, 0)

        def redo_out(r, carry):
            rs = pl.ds(pl.multiple_of(r * 128, 128), 128)
            o_ref[rs, :] = (acc_ref[rs, :] + jax.lax.dot_general(
                ot_ref[:, rs], wo_ref[...], _TN,
                preferred_element_type=f32)).astype(o_ref.dtype)
            return carry

        jax.lax.fori_loop(0, tq // 128, redo_out, 0)


@jax.jit
def pallas_parallel_sum__grouped_kv_mqa__dense_activation_silu__prompt_kernel(
    A_x: jax.Array,
    A_wq: jax.Array,
    A_wk: jax.Array,
    A_wv: jax.Array,
    A_wo: jax.Array,
    B_x: jax.Array,
    B_w1: jax.Array,
    B_w2: jax.Array,
):
    del B_x
    b, seq, d = A_x.shape
    assert b == 1
    dh = A_wk.shape[1]
    ff = B_w1.shape[1]
    hd = _H * dh
    assert A_wq.shape == (d, hd) and seq % _TQ == 0 and ff % _FC == 0
    bf16, f32 = jnp.bfloat16, jnp.float32

    def full(shape):
        return pl.BlockSpec(shape, lambda i: (0,) * len(shape))

    hbm = pl.BlockSpec(memory_space=pl.ANY)

    out = pl.pallas_call(
        functools.partial(_kernel, seq=seq, dh=dh),
        grid=(seq // _TQ,),
        in_specs=[
            hbm,
            hbm,
            hbm,
            hbm,
            hbm,
            hbm,
            hbm,
        ],
        out_specs=pl.BlockSpec((_TQ, d), lambda i: (i, 0)),
        out_shape=jax.ShapeDtypeStruct((seq, d), A_x.dtype),
        scratch_shapes=[
            pltpu.VMEM((seq, d), bf16),
            pltpu.VMEM((d, hd), bf16),
            pltpu.VMEM((hd, d), bf16),
            pltpu.VMEM((d, ff), bf16),
            pltpu.VMEM((ff, d), bf16),
            pltpu.SemaphoreType.DMA((len(_XSPLIT) + 6,)),
            pltpu.VMEM((hd + 2 * dh, d), bf16),
            pltpu.VMEM((dh, seq), f32),
            pltpu.VMEM((seq, d), bf16),
            pltpu.VMEM((seq // 2, dh), jnp.uint32),
            pltpu.VMEM((dh // 2, seq), jnp.uint32),
            pltpu.VMEM((seq // _TQ, hd, _TQ), bf16),
            pltpu.VMEM((hd, _TQ), bf16),
            pltpu.VMEM((_NKB, dh, max(_G * 16, 8), 128), f32),
            pltpu.VMEM((dh, _TQ), f32),
            pltpu.VMEM((1, _TQ), f32),
            pltpu.VMEM((seq, _TQ), f32),
            pltpu.VMEM((_TQ, max(128 * _NFB, 128)), bf16),
            pltpu.VMEM((_TQ, d), f32),
        ] + [pltpu.VMEM((_NQF, dh, _TQ), f32)] * _U
        + [pltpu.VMEM((max(_G * 16, 8), _TQ), f32)] * _U,
        compiler_params=pltpu.CompilerParams(
            dimension_semantics=("arbitrary",),
            vmem_limit_bytes=110 * 1024 * 1024,
        ),
    )(A_x.reshape(seq, d), A_wq, A_wk.T, A_wv.T, A_wo, B_w1, B_w2)
    return out.reshape(b, seq, d)
```

```python
import functools
import math

import jax
import jax.numpy as jnp
from jax.experimental import pallas as pl
from jax.experimental.pallas import tpu as pltpu

_H = 32
_EPS = 1e-5
_TQ = 512
_KC = 128
_U = 16
_W = 256
_L = 3
_LEAD = 10
_NFB = 1
_FEND = 3
_PG = 2
_PN = 3
_QAT = (0, 1, 3, 5)
_SC = 256
_QA, _KA = 127.0, 254.0
_TINY = 1e-30
_RHO_MAX = 32.0
_L_MIN, _L_MAX = 2.0 ** -40, 2.0 ** 64
_V_MIN, _V_MAX = 2.0 ** -30, 2.0 ** 60
_FC = 256
_XSPLIT = (0, 256, 512, 1024, 1536)
_LNR = 256

_NT = (((1,), (1,)), ((), ()))
_TN = (((0,), (0,)), ((), ()))


def _limbs(t16):
    b = pltpu.bitcast(t16 + (12582912.0 + 8.0), jnp.int32)
    return b >> 4, (b & 15) - 8, (b + 120) >> 8


def _recip(x):
    r = pl.reciprocal(x, approx=True)
    return r * (2.0 - x * r)


def _kernel(x_hbm, wq_hbm, wkt_hbm, wvt_hbm, wo_hbm, w1_hbm, w2_hbm, o_ref,
            x_ref, wq_ref, wo_ref, w1_ref, w2_ref, sems, wqkvt_ref, kt_ref,
            xn_ref, k8_ref, kap_ref, vt_ref, qt_ref, ot_ref, z_ref, vok_ref,
            s_ref, h_ref, acc_ref, q8_ref, cs_ref, *, seq, dh):
    f32, bf16 = jnp.float32, jnp.bfloat16
    tq, kc, U = _TQ, _KC, _U
    nc = seq // kc
    nb = _H // U
    ff = w1_ref.shape[1]
    i = pl.program_id(0)
    row0 = pl.multiple_of(i * tq, tq)
    scale = (dh ** -0.5) * math.log2(math.e)

    xb = list(_XSPLIT) + [seq]
    nx = len(_XSPLIT)
    rot = lambda r: (r + tq) % seq
    assert seq - tq in _XSPLIT
    x_copies = [
        pltpu.make_async_copy(x_hbm.at[rot(a):rot(a) + b - a],
                              x_ref.at[rot(a):rot(a) + b - a], sems.at[n])
        for n, (a, b) in enumerate(zip(xb[:-1], xb[1:]))]
    w_copies = [
        pltpu.make_async_copy(src, dst, sems.at[nx + n])
        for n, (src, dst) in enumerate(
            [(w1_hbm, w1_ref), (w2_hbm, w2_ref), (wo_hbm, wo_ref)])]
    wq_copies = [
        pltpu.make_async_copy(src, dst, sems.at[nx + 3 + n])
        for n, (src, dst) in enumerate(
            [(wq_hbm, wq_ref), (wkt_hbm, wqkvt_ref.at[0:dh]),
             (wvt_hbm, wqkvt_ref.at[dh:2 * dh])])]

    fr = tq // nb
    nw = tq // _W
    kg = _PG * kc
    ng = seq // kg

    def silu2(h):
        return (h + h * jnp.tanh(h)).astype(bf16)

    def prep_queries(q_ref, a=0, b=tq):
        for h in range(_H):
            q = q_ref[h * dh:(h + 1) * dh, :] * kap_ref[:, a:b]
            rho = jnp.maximum(
                jnp.max(jnp.abs(q), axis=0, keepdims=True), _TINY)
            qi, dq, qc = _limbs(q * ((16.0 * _QA) * _recip(rho)))
            q8_ref[h * 4 * dh:(h + 1) * 4 * dh, a:b] = jnp.concatenate(
                [qi, qi, dq, qc], axis=0).astype(jnp.int8)
            cs_ref[h:h + 1, a:b] = rho * (1.0 / (_QA * _KA))

    def heads_fast(q8all, csall, frows, arows):
        l8 = {(u, w): jnp.zeros((8, _W), f32)
              for u in range(U) for w in range(nw)}
        o = {(u, w): z_ref[:, 0:_W] for u in range(U) for w in range(nw)}
        pms, outs, oks = {}, {}, {}

        def scores(u, g, w):
            cols = slice(w * _W, (w + 1) * _W)
            t = jnp.dot(k8_ref[g * kg:(g + 1) * kg, 0:4 * dh],
                        q8all[u * 4 * dh:(u + 1) * 4 * dh, cols],
                        preferred_element_type=jnp.int32)
            pms[(u, g, w)] = jnp.exp2(t.astype(f32) * csall[u:u + 1, cols])

        def pv_mm(u, g, w):
            pm = pms.pop((u, g, w))
            for e in range(_PG):
                p = pm[e * kc:(e + 1) * kc]
                for r in range(kc // 8):
                    l8[(u, w)] = l8[(u, w)] + p[r * 8:(r + 1) * 8]
                p = jnp.concatenate(
                    [p[n * 16:(n + 1) * 16] for n in reversed(range(kc // 16))],
                    axis=0)
                ks = slice(g * kg + e * kc, g * kg + (e + 1) * kc)
                o[(u, w)] = o[(u, w)] + jnp.dot(
                    pltpu.bitcast(vt_ref[:, ks], bf16), p.astype(bf16),
                    preferred_element_type=f32)
            if g == ng - 1:
                l = jnp.sum(l8[(u, w)], axis=0, keepdims=True)
                outs[(u, w)] = (o[(u, w)] / l).astype(bf16)
                okl = jnp.logical_and(l >= _L_MIN, l <= _L_MAX)
                oks[w] = jnp.logical_and(oks[w], okl) if w in oks else okl

        def ffn_mm(k):
            fs = slice(k * 128, (k + 1) * 128)
            h_ref[arows, fs] = silu2(0.5 * jnp.dot(
                xn_ref[frows, :], w1_ref[:, fs], preferred_element_type=f32))

        items = [(u, g, w) for u in range(U) for g in range(ng)
                 for w in range(nw)]
        for t in range(len(items) + _L):
            if t < len(items):
                scores(*items[t])
            if t == len(items) + _L - _FEND:
                for k in range(_NFB):
                    ffn_mm(k)
            if t >= _L:
                pv_mm(*items[t - _L])
        ok = jnp.logical_and(
            jnp.concatenate([jnp.where(oks[w], 1.0, 0.0) for w in range(nw)],
                            axis=1) > 0.5,
            jnp.max(csall, axis=0, keepdims=True) <= _RHO_MAX / (_QA * _KA))
        ot = jnp.concatenate(
            [jnp.concatenate([outs[(u, w)] for w in range(nw)], axis=1)
             for u in range(U)], axis=0)
        return ot, jnp.where(ok, 1.0, 0.0)

    @pl.when(i == 0)
    def _():
        x_copies[0].start()
        for cp in wq_copies:
            cp.start()
        z_ref[...] = jnp.zeros(z_ref.shape, f32)

        def layernorm(a, b):
            if a in _XSPLIT and a != _LNR:
                x_copies[_XSPLIT.index(a)].wait()
                if a == 0:
                    for cp in x_copies[1:]:
                        cp.start()
                if a == _XSPLIT[-1]:
                    for cp in w_copies:
                        cp.start()
            a, b = rot(a), rot(a) + b - a
            x = x_ref[a:b, :].astype(f32)
            mu = jnp.mean(x, axis=-1, keepdims=True)
            xc = x - mu
            var = jnp.mean(xc * xc, axis=-1, keepdims=True)
            xn_ref[a:b, :] = (xc * jax.lax.rsqrt(var + _EPS)).astype(bf16)

        def project_kv(a, b):
            a, b = rot(a), rot(a) + b - a
            kv = jax.lax.dot_general(
                wqkvt_ref[0:2 * dh, :], xn_ref[a:b, :], _NT,
                preferred_element_type=f32)
            kt_ref[:, a:b] = kv[0:dh]
            vt_ref[:, a:b] = pltpu.bitcast(kv[dh:].astype(bf16), jnp.uint32)

        def project_q(a, b):
            a, b = rot(a), rot(a) + b - a
            q = jax.lax.dot_general(
                wqkvt_ref[2 * dh:, :], xn_ref[a:b, :], _NT,
                preferred_element_type=f32)
            qt_ref[a // tq, :, a % tq:a % tq + b - a] = q
            if b <= tq:
                prep_queries(q, a, b)

        edges = list(range(0, seq + 1, _LNR))
        spans = list(zip(edges[:-1], edges[1:]))
        layernorm(*spans[0])
        for cp in wq_copies:
            cp.wait()
        x_copies[1].wait()
        wqkvt_ref[2 * dh:, :] = wq_ref[...].T
        nq_done = 0
        for n, span in enumerate(spans):
            if n + 1 < len(spans):
                layernorm(*spans[n + 1])
            project_kv(*span)
            if n in _QAT:
                project_q(*spans[nq_done])
                nq_done += 1

        kt = kt_ref[...]
        kap = jnp.maximum(jnp.max(jnp.abs(kt), axis=1, keepdims=True), _TINY)
        kap_ref[...] = jnp.broadcast_to(kap * scale, kap_ref.shape)
        ki, dk, kcs = _limbs(kt * ((16.0 * _KA) / kap))
        k1 = ki >> 1
        zero = jnp.zeros_like(ki)
        kl = jnp.concatenate([k1, ki - k1, kcs, dk] + [zero] * 4, axis=0)
        for c in range(nc):
            kc32 = kl[:, c * kc:(c + 1) * kc].T
            k8_ref[c * kc:(c + 1) * kc, :] = jnp.concatenate(
                [kc32[g * 16:(g + 1) * 16] for g in reversed(range(kc // 16))],
                axis=0).astype(jnp.int8)

        vmax = jnp.max(jnp.abs(pltpu.bitcast(vt_ref[...], bf16).astype(f32)),
                       keepdims=True)
        vok = jnp.logical_and(vmax >= _V_MIN, vmax <= _V_MAX)
        vok_ref[...] = jnp.broadcast_to(jnp.where(vok, 1.0, 0.0), vok_ref.shape)
        for span in spans[nq_done:]:
            project_q(*span)
        w_copies[0].wait()

    def body(j, carry):
        rows = pl.ds(pl.multiple_of(j * (U * dh), U * dh), U * dh)
        ot, ok = heads_fast(
                            q8_ref[pl.ds(pl.multiple_of(j * (U * 4 * dh), U * 4 * dh), U * 4 * dh), :],
                            cs_ref[pl.ds(pl.multiple_of(j * U, U), U), :],
                            pl.ds(pl.multiple_of(row0 + j * fr, fr), fr),
                            pl.ds(pl.multiple_of(j * fr, fr), fr))
        ot_ref[rows, :] = ot
        return jnp.minimum(carry, ok)

    ok = jax.lax.fori_loop(0, nb, body, vok_ref[...])

    @pl.when(i == 0)
    def _():
        w_copies[1].wait()
        w_copies[2].wait()

    rows = pl.ds(row0, tq)
    xn = xn_ref[rows, :]
    acc = x_ref[rows, :].astype(f32)
    f_lo = 128 * _NFB
    fedges = ([0] if _NFB else []) + list(range(f_lo, ff, _FC)) + [ff]
    fspans = list(zip(fedges[:-1], fedges[1:]))

    def hidden(a, b):
        if b <= f_lo:
            return h_ref[...]
        return silu2(0.5 * jnp.dot(xn, w1_ref[:, a:b], preferred_element_type=f32))

    prep_queries(qt_ref.at[jnp.minimum(i + 1, seq // tq - 1)])
    h_next = hidden(*fspans[0])
    for n, (a, b) in enumerate(fspans):
        h = h_next
        if n + 1 < len(fspans):
            h_next = hidden(*fspans[n + 1])
        acc = acc + jnp.dot(h, w2_ref[a:b, :], preferred_element_type=f32)
    acc_ref[...] = acc
    o_ref[...] = (acc + jax.lax.dot_general(
        ot_ref[...], wo_ref[...], _TN,
        preferred_element_type=f32)).astype(o_ref.dtype)

    @pl.when(jnp.min(ok) < 0.5)
    def _():
        def safe_head(h, carry):
            rows = pl.ds(pl.multiple_of(h * dh, dh), dh)
            q = (qt_ref[i, rows, :] * scale).astype(bf16)

            def pass1(c, m8):
                ks = pl.ds(pl.multiple_of(c * _SC, _SC), _SC)
                s = jax.lax.dot_general(kt_ref[:, ks].astype(bf16), q, _TN,
                                        preferred_element_type=f32)
                s_ref[ks, :] = s
                return jnp.maximum(
                    m8, jnp.max(s.reshape(_SC // 8, 8, tq), axis=0))

            m8 = jax.lax.fori_loop(0, seq // _SC, pass1,
                                   jnp.full((8, tq), -jnp.inf, f32))
            m = jnp.max(m8, axis=0, keepdims=True)

            def pass2(c, lo):
                ks = pl.ds(pl.multiple_of(c * _SC, _SC), _SC)
                p = jnp.exp2(s_ref[ks, :] - m)
                return (lo[0] + jnp.sum(p.reshape(_SC // 8, 8, tq), axis=0),
                        lo[1] + jnp.dot(pltpu.bitcast(vt_ref[:, ks], bf16),
                                        p.astype(bf16),
                                        preferred_element_type=f32))

            l8, o = jax.lax.fori_loop(
                0, seq // _SC, pass2,
                (jnp.zeros((8, tq), f32), jnp.zeros((dh, tq), f32)))
            l = jnp.sum(l8, axis=0, keepdims=True)
            ot_ref[rows, :] = (o / l).astype(bf16)
            return carry

        jax.lax.fori_loop(0, _H, safe_head, 0)

        def redo_out(r, carry):
            rs = pl.ds(pl.multiple_of(r * 128, 128), 128)
            o_ref[rs, :] = (acc_ref[rs, :] + jax.lax.dot_general(
                ot_ref[:, rs], wo_ref[...], _TN,
                preferred_element_type=f32)).astype(o_ref.dtype)
            return carry

        jax.lax.fori_loop(0, tq // 128, redo_out, 0)


@jax.jit
def pallas_parallel_sum__grouped_kv_mqa__dense_activation_silu__prompt_kernel(
    A_x: jax.Array,
    A_wq: jax.Array,
    A_wk: jax.Array,
    A_wv: jax.Array,
    A_wo: jax.Array,
    B_x: jax.Array,
    B_w1: jax.Array,
    B_w2: jax.Array,
):
    del B_x
    b, seq, d = A_x.shape
    assert b == 1
    dh = A_wk.shape[1]
    ff = B_w1.shape[1]
    hd = _H * dh
    assert A_wq.shape == (d, hd) and seq % _TQ == 0 and dh == 16
    bf16, f32 = jnp.bfloat16, jnp.float32
    hbm = pl.BlockSpec(memory_space=pl.ANY)

    out = pl.pallas_call(
        functools.partial(_kernel, seq=seq, dh=dh),
        grid=(seq // _TQ,),
        in_specs=[hbm] * 7,
        out_specs=pl.BlockSpec((_TQ, d), lambda i: (i, 0)),
        out_shape=jax.ShapeDtypeStruct((seq, d), A_x.dtype),
        scratch_shapes=[
            pltpu.VMEM((seq, d), bf16),
            pltpu.VMEM((d, hd), bf16),
            pltpu.VMEM((hd, d), bf16),
            pltpu.VMEM((d, ff), bf16),
            pltpu.VMEM((ff, d), bf16),
            pltpu.SemaphoreType.DMA((len(_XSPLIT) + 6,)),
            pltpu.VMEM((hd + 2 * dh, d), bf16),
            pltpu.VMEM((dh, seq), f32),
            pltpu.VMEM((seq, d), bf16),
            pltpu.VMEM((seq, 128), jnp.int8),
            pltpu.VMEM((dh, _TQ), f32),
            pltpu.VMEM((dh // 2, seq), jnp.uint32),
            pltpu.VMEM((seq // _TQ, hd, _TQ), f32),
            pltpu.VMEM((hd, _TQ), bf16),
            pltpu.VMEM((dh, _TQ), f32),
            pltpu.VMEM((1, _TQ), f32),
            pltpu.VMEM((seq, _TQ), f32),
            pltpu.VMEM((_TQ, max(128 * _NFB, 128)), bf16),
            pltpu.VMEM((_TQ, d), f32),
            pltpu.VMEM((4 * hd, _TQ), jnp.int8),
            pltpu.VMEM((_H, _TQ), f32),
        ],
        compiler_params=pltpu.CompilerParams(
            dimension_semantics=("arbitrary",),
            vmem_limit_bytes=100 * 1024 * 1024,
        ),
    )(A_x.reshape(seq, d), A_wq, A_wk.T, A_wv.T, A_wo, B_w1, B_w2)
    return out.reshape(b, seq, d)
```

```python
import functools
import math

import jax
import jax.numpy as jnp
from jax.experimental import pallas as pl
from jax.experimental.pallas import tpu as pltpu

_H = 32
_EPS = 1e-5
_TQ = 512
_KC = 128
_PG = 2
_W = 256
_LAG = 3
_U = 16
_F0 = 128
_FC = 512
_SC = 256
_LNR = 256

_QA, _KA = 127.0, 254.0
_TINY = 1e-30
_RHO_MAX = 32.0
_L_MIN, _L_MAX = 2.0 ** -40, 2.0 ** 64
_V_MIN, _V_MAX = 2.0 ** -30, 2.0 ** 60

_XSPLIT = (0, 256, 512, 1024, 1536)
_XWAIT = {0: (0,), 512: (2,), 1024: (3, 4)}
_PRO = (("ln", 1), ("kq", 0), ("ln", 2), ("kq", 1), ("ln", 3), ("kq", 2),
        ("ln", 4), ("ln", 5), ("kq", 3), ("ln", 6), ("ln", 7), ("kq", 4),
        ("k", 6), ("k", 7), ("kq", 5))
_PRO_Q = (6, 7)

_NT = (((1,), (1,)), ((), ()))
_TN = (((0,), (0,)), ((), ()))


def _limbs(t16):
    b = pltpu.bitcast(t16 + (12582912.0 + 8.0), jnp.int32)
    return b >> 4, (b & 15) - 8, (b + 120) >> 8


def _recip(x):
    r = pl.reciprocal(x, approx=True)
    return r * (2.0 - x * r)


def _silu2(h):
    return (h + h * jnp.tanh(h)).astype(jnp.bfloat16)


def _kernel(x_hbm, wq_hbm, wkt_hbm, wvt_hbm, wo_hbm, w1_hbm, w2_hbm, o_ref,
            x_ref, wq_ref, wo_ref, w1_ref, w2_ref, sems, wt_ref, kt_ref,
            xn_ref, k8_ref, kap_ref, vt_ref, qt_ref, ot_ref, z_ref, vok_ref,
            s_ref, h_ref, acc_ref, q8_ref, cs_ref, *, seq, dh):
    f32, bf16 = jnp.float32, jnp.bfloat16
    tq, kc = _TQ, _KC
    nb = _H // _U
    fr = tq // nb
    nw = tq // _W
    kg = _PG * kc
    ng = seq // kg
    ff = w1_ref.shape[1]
    i = pl.program_id(0)
    row0 = pl.multiple_of(i * tq, tq)
    scale = (dh ** -0.5) * math.log2(math.e)

    def rot(r):
        return (r + tq) % seq

    xb = list(_XSPLIT) + [seq]
    nx = len(_XSPLIT)
    x_copies = [
        pltpu.make_async_copy(x_hbm.at[rot(a):rot(a) + b - a],
                              x_ref.at[rot(a):rot(a) + b - a], sems.at[n])
        for n, (a, b) in enumerate(zip(xb[:-1], xb[1:]))]
    w_copies = [
        pltpu.make_async_copy(src, dst, sems.at[nx + n])
        for n, (src, dst) in enumerate(
            [(w1_hbm.at[:, 0:_F0], w1_ref.at[:, 0:_F0]),
             (w1_hbm.at[:, _F0:], w1_ref.at[:, _F0:]),
             (w2_hbm, w2_ref), (wo_hbm, wo_ref)])]
    wq_copies = [
        pltpu.make_async_copy(src, dst, sems.at[nx + 4 + n])
        for n, (src, dst) in enumerate(
            [(wq_hbm, wq_ref), (wkt_hbm, wt_ref.at[0:dh]),
             (wvt_hbm, wt_ref.at[dh:2 * dh])])]

    def prep_queries(qt, a=0, b=tq):
        for h in range(_H):
            q = qt[h * dh:(h + 1) * dh, :] * kap_ref[:, a:b]
            rho = jnp.maximum(
                jnp.max(jnp.abs(q), axis=0, keepdims=True), _TINY)
            qi, dq, qc = _limbs(q * ((16.0 * _QA) * _recip(rho)))
            q8_ref[h * 4 * dh:(h + 1) * 4 * dh, a:b] = jnp.concatenate(
                [qi, qi, dq, qc], axis=0).astype(jnp.int8)
            cs_ref[h:h + 1, a:b] = rho * (1.0 / (_QA * _KA))

    @pl.when(i == 0)
    def _():
        x_copies[0].start()
        for cp in wq_copies:
            cp.start()
        z_ref[...] = jnp.zeros(z_ref.shape, f32)

        def layernorm(n):
            a = n * _LNR
            if a in _XWAIT:
                for c in _XWAIT[a]:
                    x_copies[c].wait()
                if a == 0:
                    for cp in x_copies[1:]:
                        cp.start()
                if a == max(_XWAIT):
                    for cp in w_copies:
                        cp.start()
            a, b = rot(a), rot(a) + _LNR
            x = x_ref[a:b, :].astype(f32)
            mu = jnp.mean(x, axis=-1, keepdims=True)
            xc = x - mu
            var = jnp.mean(xc * xc, axis=-1, keepdims=True)
            xn_ref[a:b, :] = (xc * jax.lax.rsqrt(var + _EPS)).astype(bf16)

        def project(n, want_kv, want_q):
            a, b = rot(n * _LNR), rot(n * _LNR) + _LNR
            lo = 0 if want_kv else 2 * dh
            hi = 2 * dh + (_H * dh if want_q else 0)
            r = jax.lax.dot_general(wt_ref[lo:hi, :], xn_ref[a:b, :], _NT,
                                    preferred_element_type=f32)
            if want_kv:
                kt_ref[:, a:b] = r[0:dh]
                vt_ref[:, a:b] = pltpu.bitcast(
                    r[dh:2 * dh].astype(bf16), jnp.uint32)
            if want_q:
                q = r[2 * dh - lo:]
                qt_ref[a // tq, :, a % tq:a % tq + _LNR] = q
                if b <= tq:
                    prep_queries(q, a, b)

        layernorm(0)
        for cp in wq_copies:
            cp.wait()
        x_copies[1].wait()
        wt_ref[2 * dh:, :] = wq_ref[...].T
        for op, n in _PRO:
            if op == "ln":
                layernorm(n)
            else:
                project(n, "k" in op, "q" in op)

        kt = kt_ref[...]
        kap = jnp.maximum(jnp.max(jnp.abs(kt), axis=1, keepdims=True), _TINY)
        kap_ref[...] = jnp.broadcast_to(kap * scale, kap_ref.shape)
        ki, dk, kcs = _limbs(kt * ((16.0 * _KA) / kap))
        k1 = ki >> 1
        zero = jnp.zeros_like(ki)
        kl = jnp.concatenate([k1, ki - k1, kcs, dk] + [zero] * 4, axis=0)
        for c in range(seq // kc):
            kcl = kl[:, c * kc:(c + 1) * kc].T
            k8_ref[c * kc:(c + 1) * kc, :] = jnp.concatenate(
                [kcl[g * 16:(g + 1) * 16] for g in reversed(range(kc // 16))],
                axis=0).astype(jnp.int8)

        vmax = jnp.max(jnp.abs(pltpu.bitcast(vt_ref[...], bf16).astype(f32)),
                       keepdims=True)
        vok = jnp.logical_and(vmax >= _V_MIN, vmax <= _V_MAX)
        vok_ref[...] = jnp.broadcast_to(jnp.where(vok, 1.0, 0.0), vok_ref.shape)
        for n in _PRO_Q:
            project(n, False, True)
        w_copies[0].wait()

    def heads(j, ok_in):
        q8 = q8_ref[pl.ds(pl.multiple_of(j * (_U * 4 * dh), _U * 4 * dh),
                          _U * 4 * dh), :]
        cs = cs_ref[pl.ds(pl.multiple_of(j * _U, _U), _U), :]
        uw = [(u, w) for u in range(_U) for w in range(nw)]
        l8 = {k: jnp.zeros((8, _W), f32) for k in uw}
        o = {k: z_ref[...] for k in uw}
        ps, outs, oks = {}, {}, {}

        def scores(u, g, w):
            cols = slice(w * _W, (w + 1) * _W)
            t = jnp.dot(k8_ref[g * kg:(g + 1) * kg, 0:4 * dh],
                        q8[u * 4 * dh:(u + 1) * 4 * dh, cols],
                        preferred_element_type=jnp.int32)
            ps[(u, g, w)] = jnp.exp2(t.astype(f32) * cs[u:u + 1, cols])

        def pv(u, g, w):
            pg = ps.pop((u, g, w))
            for e in range(_PG):
                p = pg[e * kc:(e + 1) * kc]
                for r in range(kc // 8):
                    l8[(u, w)] = l8[(u, w)] + p[r * 8:(r + 1) * 8]
                p = jnp.concatenate(
                    [p[n * 16:(n + 1) * 16] for n in reversed(range(kc // 16))],
                    axis=0)
                ks = slice(g * kg + e * kc, g * kg + (e + 1) * kc)
                o[(u, w)] = o[(u, w)] + jnp.dot(
                    pltpu.bitcast(vt_ref[:, ks], bf16), p.astype(bf16),
                    preferred_element_type=f32)
            if g == ng - 1:
                l = jnp.sum(l8[(u, w)], axis=0, keepdims=True)
                outs[(u, w)] = (o[(u, w)] / l).astype(bf16)
                okl = jnp.logical_and(l >= _L_MIN, l <= _L_MAX)
                oks[w] = jnp.logical_and(oks[w], okl) if w in oks else okl

        items = [(u, g, w) for u in range(_U) for g in range(ng)
                 for w in range(nw)]
        for t in range(len(items) + _LAG):
            if t < len(items):
                scores(*items[t])
            if t == len(items):
                rows = pl.ds(pl.multiple_of(row0 + j * fr, fr), fr)
                h_ref[pl.ds(pl.multiple_of(j * fr, fr), fr), :] = _silu2(
                    0.5 * jnp.dot(xn_ref[rows, :], w1_ref[:, 0:_F0],
                                  preferred_element_type=f32))
            if t >= _LAG:
                pv(*items[t - _LAG])

        ot_ref[pl.ds(pl.multiple_of(j * (_U * dh), _U * dh), _U * dh), :] = (
            jnp.concatenate(
                [jnp.concatenate([outs[(u, w)] for w in range(nw)], axis=1)
                 for u in range(_U)], axis=0))
        ok = jnp.concatenate(
            [jnp.where(oks[w], 1.0, 0.0) for w in range(nw)], axis=1)
        rho_ok = jnp.max(cs, axis=0, keepdims=True) <= _RHO_MAX / (_QA * _KA)
        return jnp.minimum(ok_in, jnp.where(rho_ok, ok, 0.0))

    ok = jax.lax.fori_loop(0, nb, heads, vok_ref[...])

    @pl.when(i == 0)
    def _():
        for cp in w_copies[1:]:
            cp.wait()

    rows = pl.ds(row0, tq)
    xn = xn_ref[rows, :]
    acc = x_ref[rows, :].astype(f32)
    fedges = [0] + list(range(_F0, ff, _FC)) + [ff]
    fspans = list(zip(fedges[:-1], fedges[1:]))

    def hidden(a, b):
        if a == 0:
            return h_ref[...]
        return _silu2(0.5 * jnp.dot(xn, w1_ref[:, a:b],
                                    preferred_element_type=f32))

    prep_queries(qt_ref.at[jnp.minimum(i + 1, seq // tq - 1)])
    h_next = hidden(*fspans[0])
    for n, (a, b) in enumerate(fspans):
        h = h_next
        if n + 1 < len(fspans):
            h_next = hidden(*fspans[n + 1])
        acc = acc + jnp.dot(h, w2_ref[a:b, :], preferred_element_type=f32)
    acc_ref[...] = acc
    o_ref[...] = (acc + jax.lax.dot_general(
        ot_ref[...], wo_ref[...], _TN,
        preferred_element_type=f32)).astype(o_ref.dtype)

    @pl.when(jnp.min(ok) < 0.5)
    def _():
        def safe_head(h, carry):
            hr = pl.ds(pl.multiple_of(h * dh, dh), dh)
            q = (qt_ref[i, hr, :] * scale).astype(bf16)

            def pass1(c, m8):
                ks = pl.ds(pl.multiple_of(c * _SC, _SC), _SC)
                s = jax.lax.dot_general(kt_ref[:, ks].astype(bf16), q, _TN,
                                        preferred_element_type=f32)
                s_ref[ks, :] = s
                return jnp.maximum(
                    m8, jnp.max(s.reshape(_SC // 8, 8, tq), axis=0))

            m8 = jax.lax.fori_loop(0, seq // _SC, pass1,
                                   jnp.full((8, tq), -jnp.inf, f32))
            m = jnp.max(m8, axis=0, keepdims=True)

            def pass2(c, lo):
                ks = pl.ds(pl.multiple_of(c * _SC, _SC), _SC)
                p = jnp.exp2(s_ref[ks, :] - m)
                return (lo[0] + jnp.sum(p.reshape(_SC // 8, 8, tq), axis=0),
                        lo[1] + jnp.dot(pltpu.bitcast(vt_ref[:, ks], bf16),
                                        p.astype(bf16),
                                        preferred_element_type=f32))

            l8, o = jax.lax.fori_loop(
                0, seq // _SC, pass2,
                (jnp.zeros((8, tq), f32), jnp.zeros((dh, tq), f32)))
            l = jnp.sum(l8, axis=0, keepdims=True)
            ot_ref[hr, :] = (o / l).astype(bf16)
            return carry

        jax.lax.fori_loop(0, _H, safe_head, 0)

        def redo_out(r, carry):
            rs = pl.ds(pl.multiple_of(r * 128, 128), 128)
            o_ref[rs, :] = (acc_ref[rs, :] + jax.lax.dot_general(
                ot_ref[:, rs], wo_ref[...], _TN,
                preferred_element_type=f32)).astype(o_ref.dtype)
            return carry

        jax.lax.fori_loop(0, tq // 128, redo_out, 0)


@jax.jit
def pallas_parallel_sum__grouped_kv_mqa__dense_activation_silu__prompt_kernel(
    A_x: jax.Array,
    A_wq: jax.Array,
    A_wk: jax.Array,
    A_wv: jax.Array,
    A_wo: jax.Array,
    B_x: jax.Array,
    B_w1: jax.Array,
    B_w2: jax.Array,
):
    del B_x
    b, seq, d = A_x.shape
    dh = A_wk.shape[1]
    ff = B_w1.shape[1]
    hd = _H * dh
    assert b == 1 and seq == 8 * _LNR == 4 * _TQ and dh == 16
    assert A_wq.shape == (d, hd) and ff % 128 == 0
    bf16, f32 = jnp.bfloat16, jnp.float32

    out = pl.pallas_call(
        functools.partial(_kernel, seq=seq, dh=dh),
        grid=(seq // _TQ,),
        in_specs=[pl.BlockSpec(memory_space=pl.ANY)] * 7,
        out_specs=pl.BlockSpec((_TQ, d), lambda i: (i, 0)),
        out_shape=jax.ShapeDtypeStruct((seq, d), A_x.dtype),
        scratch_shapes=[
            pltpu.VMEM((seq, d), bf16),
            pltpu.VMEM((d, hd), bf16),
            pltpu.VMEM((hd, d), bf16),
            pltpu.VMEM((d, ff), bf16),
            pltpu.VMEM((ff, d), bf16),
            pltpu.SemaphoreType.DMA((len(_XSPLIT) + 7,)),
            pltpu.VMEM((hd + 2 * dh, d), bf16),
            pltpu.VMEM((dh, seq), f32),
            pltpu.VMEM((seq, d), bf16),
            pltpu.VMEM((seq, 128), jnp.int8),
            pltpu.VMEM((dh, _TQ), f32),
            pltpu.VMEM((dh // 2, seq), jnp.uint32),
            pltpu.VMEM((seq // _TQ, hd, _TQ), f32),
            pltpu.VMEM((hd, _TQ), bf16),
            pltpu.VMEM((dh, _W), f32),
            pltpu.VMEM((1, _TQ), f32),
            pltpu.VMEM((seq, _TQ), f32),
            pltpu.VMEM((_TQ, _F0), bf16),
            pltpu.VMEM((_TQ, d), f32),
            pltpu.VMEM((4 * hd, _TQ), jnp.int8),
            pltpu.VMEM((_H, _TQ), f32),
        ],
        compiler_params=pltpu.CompilerParams(
            dimension_semantics=("arbitrary",),
            vmem_limit_bytes=64 * 1024 * 1024,
        ),
    )(A_x.reshape(seq, d), A_wq, A_wk.T, A_wv.T, A_wo, B_w1, B_w2)
    return out.reshape(b, seq, d)
```

```python
import functools
import math

import jax
import jax.numpy as jnp
from jax.experimental import pallas as pl
from jax.experimental.pallas import tpu as pltpu

_H = 32
_EPS = 1e-5
_TQ = 512
_KC = 128
_PG = 2
_W = 256
_LAG = 3
_U = 16
_F0 = 128
_FC = 512
_SC = 256
_LNR = 256

_QA, _KA = 127.0, 254.0
_TINY = 1e-30
_RHO_MAX = 32.0
_L_MIN, _L_MAX = 2.0 ** -40, 2.0 ** 64
_V_MIN, _V_MAX = 2.0 ** -30, 2.0 ** 60

_XSPLIT = (0, 256, 512, 1024, 1536)
_XWAIT = {0: (0,), 512: (2,), 1024: (3, 4)}
_PRO = (("ln", 1), ("kq", 0), ("ln", 2), ("kq", 1), ("ln", 3), ("kq", 2),
        ("ln", 4), ("ln", 5), ("kq", 3), ("ln", 6), ("ln", 7), ("kq", 4),
        ("k", 6), ("k", 7), ("kq", 5))
_PRO_Q = (6, 7)

_NT = (((1,), (1,)), ((), ()))
_TN = (((0,), (0,)), ((), ()))


def _limbs(t16):
    b = pltpu.bitcast(t16 + (12582912.0 + 8.0), jnp.int32)
    return b >> 4, (b & 15) - 8, (b + 120) >> 8


def _recip(x):
    r = pl.reciprocal(x, approx=True)
    return r * (2.0 - x * r)


def _silu2(h):
    return (h + h * jnp.tanh(h)).astype(jnp.bfloat16)


def _kernel(x_hbm, wq_hbm, wkt_hbm, wvt_hbm, wo_hbm, w1_hbm, w2_hbm, o_ref,
            x_ref, wq_ref, wo_ref, w1_ref, w2_ref, sems, wt_ref, kt_ref,
            xn_ref, k8_ref, kap_ref, vt_ref, qt_ref, ot_ref, z_ref, vok_ref,
            s_ref, h_ref, acc_ref, q8_ref, cs_ref, *, seq, dh):
    f32, bf16 = jnp.float32, jnp.bfloat16
    tq, kc = _TQ, _KC
    nb = _H // _U
    fr = tq // nb
    nw = tq // _W
    kg = _PG * kc
    ng = seq // kg
    ff = w1_ref.shape[1]
    i = pl.program_id(0)
    row0 = pl.multiple_of(i * tq, tq)
    scale = (dh ** -0.5) * math.log2(math.e)

    def rot(r):
        return (r + tq) % seq

    xb = list(_XSPLIT) + [seq]
    nx = len(_XSPLIT)
    x_copies = [
        pltpu.make_async_copy(x_hbm.at[rot(a):rot(a) + b - a],
                              x_ref.at[rot(a):rot(a) + b - a], sems.at[n])
        for n, (a, b) in enumerate(zip(xb[:-1], xb[1:]))]
    w_copies = [
        pltpu.make_async_copy(src, dst, sems.at[nx + n])
        for n, (src, dst) in enumerate(
            [(w1_hbm.at[:, 0:_F0], w1_ref.at[:, 0:_F0]),
             (w1_hbm.at[:, _F0:], w1_ref.at[:, _F0:]),
             (w2_hbm, w2_ref), (wo_hbm, wo_ref)])]
    wq_copies = [
        pltpu.make_async_copy(src, dst, sems.at[nx + 4 + n])
        for n, (src, dst) in enumerate(
            [(wq_hbm, wq_ref), (wkt_hbm, wt_ref.at[0:dh]),
             (wvt_hbm, wt_ref.at[dh:2 * dh])])]

    def prep_queries(qt, a=0, b=tq, hs=range(_H), after=None):
        for h in hs:
            kap = kap_ref[:, a:b]
            if after is not None:
                kap = kap + after(h) * 0.0
            q = qt[h * dh:(h + 1) * dh, :] * kap
            rho = jnp.maximum(
                jnp.max(jnp.abs(q), axis=0, keepdims=True), _TINY)
            qi, dq, qc = _limbs(q * ((16.0 * _QA) * _recip(rho)))
            q8_ref[h * 4 * dh:(h + 1) * 4 * dh, a:b] = jnp.concatenate(
                [qi, qi, dq, qc], axis=0).astype(jnp.int8)
            cs_ref[h:h + 1, a:b] = rho * (1.0 / (_QA * _KA))

    @pl.when(i == 0)
    def _():
        x_copies[0].start()
        for cp in wq_copies:
            cp.start()
        z_ref[...] = jnp.zeros(z_ref.shape, f32)

        def layernorm(n):
            a = n * _LNR
            if a in _XWAIT:
                for c in _XWAIT[a]:
                    x_copies[c].wait()
                if a == 0:
                    for cp in x_copies[1:]:
                        cp.start()
                if a == max(_XWAIT):
                    for cp in w_copies:
                        cp.start()
            a, b = rot(a), rot(a) + _LNR
            x = x_ref[a:b, :].astype(f32)
            mu = jnp.mean(x, axis=-1, keepdims=True)
            xc = x - mu
            var = jnp.mean(xc * xc, axis=-1, keepdims=True)
            xn_ref[a:b, :] = (xc * jax.lax.rsqrt(var + _EPS)).astype(bf16)

        def project(n, want_kv, want_q):
            a, b = rot(n * _LNR), rot(n * _LNR) + _LNR
            lo = 0 if want_kv else 2 * dh
            hi = 2 * dh + (_H * dh if want_q else 0)
            r = jax.lax.dot_general(wt_ref[lo:hi, :], xn_ref[a:b, :], _NT,
                                    preferred_element_type=f32)
            if want_kv:
                kt_ref[:, a:b] = r[0:dh]
                vt_ref[:, a:b] = pltpu.bitcast(
                    r[dh:2 * dh].astype(bf16), jnp.uint32)
            if want_q:
                q = r[2 * dh - lo:]
                qt_ref[a // tq, :, a % tq:a % tq + _LNR] = q
                if b <= tq:
                    prep_queries(q, a, b)

        layernorm(0)
        for cp in wq_copies:
            cp.wait()
        x_copies[1].wait()
        wt_ref[2 * dh:, :] = wq_ref[...].T
        for op, n in _PRO:
            if op == "ln":
                layernorm(n)
            else:
                project(n, "k" in op, "q" in op)

        kt = kt_ref[...]
        kap = jnp.maximum(jnp.max(jnp.abs(kt), axis=1, keepdims=True), _TINY)
        kap_ref[...] = jnp.broadcast_to(kap * scale, kap_ref.shape)
        ki, dk, kcs = _limbs(kt * ((16.0 * _KA) / kap))
        k1 = ki >> 1
        zero = jnp.zeros_like(ki)
        kl = jnp.concatenate([k1, ki - k1, kcs, dk] + [zero] * 4, axis=0)
        for c in range(seq // kc):
            kcl = kl[:, c * kc:(c + 1) * kc].T
            k8_ref[c * kc:(c + 1) * kc, :] = jnp.concatenate(
                [kcl[g * 16:(g + 1) * 16] for g in reversed(range(kc // 16))],
                axis=0).astype(jnp.int8)

        vmax = jnp.max(jnp.abs(pltpu.bitcast(vt_ref[...], bf16).astype(f32)),
                       keepdims=True)
        vok = jnp.logical_and(vmax >= _V_MIN, vmax <= _V_MAX)
        vok_ref[...] = jnp.broadcast_to(jnp.where(vok, 1.0, 0.0), vok_ref.shape)
        for n in _PRO_Q:
            project(n, False, True)
        w_copies[0].wait()

    def heads(j, ok_in):
        q8 = q8_ref[pl.ds(pl.multiple_of(j * (_U * 4 * dh), _U * 4 * dh),
                          _U * 4 * dh), :]
        cs = cs_ref[pl.ds(pl.multiple_of(j * _U, _U), _U), :]
        uw = [(u, w) for u in range(_U) for w in range(nw)]
        l8 = {k: jnp.zeros((8, _W), f32) for k in uw}
        o = {k: z_ref[...] for k in uw}
        ps, outs, oks = {}, {}, {}

        def scores(u, g, w):
            cols = slice(w * _W, (w + 1) * _W)
            t = jnp.dot(k8_ref[g * kg:(g + 1) * kg, 0:4 * dh],
                        q8[u * 4 * dh:(u + 1) * 4 * dh, cols],
                        preferred_element_type=jnp.int32)
            ps[(u, g, w)] = jnp.exp2(t.astype(f32) * cs[u:u + 1, cols])

        def pv(u, g, w):
            pg = ps.pop((u, g, w))
            for e in range(_PG):
                p = pg[e * kc:(e + 1) * kc]
                for r in range(kc // 8):
                    l8[(u, w)] = l8[(u, w)] + p[r * 8:(r + 1) * 8]
                p = jnp.concatenate(
                    [p[n * 16:(n + 1) * 16] for n in reversed(range(kc // 16))],
                    axis=0)
                ks = slice(g * kg + e * kc, g * kg + (e + 1) * kc)
                o[(u, w)] = o[(u, w)] + jnp.dot(
                    pltpu.bitcast(vt_ref[:, ks], bf16), p.astype(bf16),
                    preferred_element_type=f32)
            if g == ng - 1:
                l = jnp.sum(l8[(u, w)], axis=0, keepdims=True)
                outs[(u, w)] = (o[(u, w)] / l).astype(bf16)
                okl = jnp.logical_and(l >= _L_MIN, l <= _L_MAX)
                oks[w] = jnp.logical_and(oks[w], okl) if w in oks else okl

        items = [(u, g, w) for u in range(_U) for g in range(ng)
                 for w in range(nw)]
        for t in range(len(items) + _LAG):
            if t < len(items):
                scores(*items[t])
            if t == len(items):
                rows = pl.ds(pl.multiple_of(row0 + j * fr, fr), fr)
                h_ref[pl.ds(pl.multiple_of(j * fr, fr), fr), :] = _silu2(
                    0.5 * jnp.dot(xn_ref[rows, :], w1_ref[:, 0:_F0],
                                  preferred_element_type=f32))
            if t >= _LAG:
                pv(*items[t - _LAG])

        ot_ref[pl.ds(pl.multiple_of(j * (_U * dh), _U * dh), _U * dh), :] = (
            jnp.concatenate(
                [jnp.concatenate([outs[(u, w)] for w in range(nw)], axis=1)
                 for u in range(_U)], axis=0))
        ok = jnp.concatenate(
            [jnp.where(oks[w], 1.0, 0.0) for w in range(nw)], axis=1)
        rho_ok = jnp.max(cs, axis=0, keepdims=True) <= _RHO_MAX / (_QA * _KA)
        return jnp.minimum(ok_in, jnp.where(rho_ok, ok, 0.0))

    ok = jax.lax.fori_loop(0, nb, heads, vok_ref[...])

    @pl.when(i == 0)
    def _():
        for cp in w_copies[1:]:
            cp.wait()

    rows = pl.ds(row0, tq)
    xn = xn_ref[rows, :]
    acc = x_ref[rows, :].astype(f32)
    fedges = [0] + list(range(_F0, ff, _FC)) + [ff]
    fspans = list(zip(fedges[:-1], fedges[1:]))
    assert len(fspans) >= _H // 8 and acc.shape == (tq, tq)

    def hidden(a, b):
        if a == 0:
            return h_ref[...]
        return _silu2(0.5 * jnp.dot(xn, w1_ref[:, a:b],
                                    preferred_element_type=f32))

    qn = qt_ref.at[jnp.minimum(i + 1, seq // tq - 1)]
    h_next = hidden(*fspans[0])
    for n, (a, b) in enumerate(fspans):
        h = h_next
        if n + 1 < len(fspans):
            h_next = hidden(*fspans[n + 1])
        acc = acc + jnp.dot(h, w2_ref[a:b, :], preferred_element_type=f32)
        if n < _H // 8:
            prep_queries(qn, hs=range(8 * n, 8 * n + 8),
                         after=lambda h: acc[(h % 8) * 64:(h % 8) * 64 + 1, :])
    acc_ref[...] = acc
    o_ref[...] = (acc + jax.lax.dot_general(
        ot_ref[...], wo_ref[...], _TN,
        preferred_element_type=f32)).astype(o_ref.dtype)

    @pl.when(jnp.min(ok) < 0.5)
    def _():
        def safe_head(h, carry):
            hr = pl.ds(pl.multiple_of(h * dh, dh), dh)
            q = (qt_ref[i, hr, :] * scale).astype(bf16)

            def pass1(c, m8):
                ks = pl.ds(pl.multiple_of(c * _SC, _SC), _SC)
                s = jax.lax.dot_general(kt_ref[:, ks].astype(bf16), q, _TN,
                                        preferred_element_type=f32)
                s_ref[ks, :] = s
                return jnp.maximum(
                    m8, jnp.max(s.reshape(_SC // 8, 8, tq), axis=0))

            m8 = jax.lax.fori_loop(0, seq // _SC, pass1,
                                   jnp.full((8, tq), -jnp.inf, f32))
            m = jnp.max(m8, axis=0, keepdims=True)

            def pass2(c, lo):
                ks = pl.ds(pl.multiple_of(c * _SC, _SC), _SC)
                p = jnp.exp2(s_ref[ks, :] - m)
                return (lo[0] + jnp.sum(p.reshape(_SC // 8, 8, tq), axis=0),
                        lo[1] + jnp.dot(pltpu.bitcast(vt_ref[:, ks], bf16),
                                        p.astype(bf16),
                                        preferred_element_type=f32))

            l8, o = jax.lax.fori_loop(
                0, seq // _SC, pass2,
                (jnp.zeros((8, tq), f32), jnp.zeros((dh, tq), f32)))
            l = jnp.sum(l8, axis=0, keepdims=True)
            ot_ref[hr, :] = (o / l).astype(bf16)
            return carry

        jax.lax.fori_loop(0, _H, safe_head, 0)

        def redo_out(r, carry):
            rs = pl.ds(pl.multiple_of(r * 128, 128), 128)
            o_ref[rs, :] = (acc_ref[rs, :] + jax.lax.dot_general(
                ot_ref[:, rs], wo_ref[...], _TN,
                preferred_element_type=f32)).astype(o_ref.dtype)
            return carry

        jax.lax.fori_loop(0, tq // 128, redo_out, 0)


@jax.jit
def pallas_parallel_sum__grouped_kv_mqa__dense_activation_silu__prompt_kernel(
    A_x: jax.Array,
    A_wq: jax.Array,
    A_wk: jax.Array,
    A_wv: jax.Array,
    A_wo: jax.Array,
    B_x: jax.Array,
    B_w1: jax.Array,
    B_w2: jax.Array,
):
    del B_x
    b, seq, d = A_x.shape
    dh = A_wk.shape[1]
    ff = B_w1.shape[1]
    hd = _H * dh
    assert b == 1 and seq == 8 * _LNR == 4 * _TQ and dh == 16
    assert A_wq.shape == (d, hd) and ff % 128 == 0
    bf16, f32 = jnp.bfloat16, jnp.float32

    out = pl.pallas_call(
        functools.partial(_kernel, seq=seq, dh=dh),
        grid=(seq // _TQ,),
        in_specs=[pl.BlockSpec(memory_space=pl.ANY)] * 7,
        out_specs=pl.BlockSpec((_TQ, d), lambda i: (i, 0)),
        out_shape=jax.ShapeDtypeStruct((seq, d), A_x.dtype),
        scratch_shapes=[
            pltpu.VMEM((seq, d), bf16),
            pltpu.VMEM((d, hd), bf16),
            pltpu.VMEM((hd, d), bf16),
            pltpu.VMEM((d, ff), bf16),
            pltpu.VMEM((ff, d), bf16),
            pltpu.SemaphoreType.DMA((len(_XSPLIT) + 7,)),
            pltpu.VMEM((hd + 2 * dh, d), bf16),
            pltpu.VMEM((dh, seq), f32),
            pltpu.VMEM((seq, d), bf16),
            pltpu.VMEM((seq, 128), jnp.int8),
            pltpu.VMEM((dh, _TQ), f32),
            pltpu.VMEM((dh // 2, seq), jnp.uint32),
            pltpu.VMEM((seq // _TQ, hd, _TQ), f32),
            pltpu.VMEM((hd, _TQ), bf16),
            pltpu.VMEM((dh, _W), f32),
            pltpu.VMEM((1, _TQ), f32),
            pltpu.VMEM((seq, _TQ), f32),
            pltpu.VMEM((_TQ, _F0), bf16),
            pltpu.VMEM((_TQ, d), f32),
            pltpu.VMEM((4 * hd, _TQ), jnp.int8),
            pltpu.VMEM((_H, _TQ), f32),
        ],
        compiler_params=pltpu.CompilerParams(
            dimension_semantics=("arbitrary",),
            vmem_limit_bytes=64 * 1024 * 1024,
        ),
    )(A_x.reshape(seq, d), A_wq, A_wk.T, A_wv.T, A_wo, B_w1, B_w2)
    return out.reshape(b, seq, d)
```

```python
import functools
import math

import jax
import jax.numpy as jnp
from jax.experimental import pallas as pl
from jax.experimental.pallas import tpu as pltpu

_H = 32
_EPS = 1e-5
_TQ = 512
_KC = 128
_PG = 2
_W = 256
_LAG = 3
_U = 16
_F0 = 128
_FC = 512
_SC = 256
_LNR = 256

_QA, _KA = 127.0, 254.0
_TINY = 1e-30
_RHO_MAX = 32.0
_L_MIN, _L_MAX = 2.0 ** -40, 2.0 ** 64
_V_MIN, _V_MAX = 2.0 ** -30, 2.0 ** 60

_XSPLIT = (0, 256, 512, 1024, 1536)
_XWAIT = {0: (0,), 512: (2,), 1024: (3, 4)}
_PRO = (("ln", 1), ("kq", 0), ("ln", 2), ("kq", 1), ("ln", 3), ("kq", 2),
        ("ln", 4), ("ln", 5), ("kq", 3), ("ln", 6), ("ln", 7), ("kq", 4),
        ("k", 6), ("k", 7), ("kq", 5))
_PRO_Q = (6, 7)

_NT = (((1,), (1,)), ((), ()))
_TN = (((0,), (0,)), ((), ()))


def _limbs(t16):
    b = pltpu.bitcast(t16 + (12582912.0 + 8.0), jnp.int32)
    return b >> 4, (b & 15) - 8, (b + 120) >> 8


def _recip(x):
    r = pl.reciprocal(x, approx=True)
    return r * (2.0 - x * r)


def _silu(h):
    return (h * jax.nn.sigmoid(h)).astype(jnp.bfloat16)


def _kernel(x_hbm, wq_hbm, wkt_hbm, wvt_hbm, wo_hbm, w1_hbm, w2_hbm, o_ref,
            x_ref, wq_ref, wo_ref, w1_ref, w2_ref, sems, wt_ref, kt_ref,
            xn_ref, k8_ref, kap_ref, vt_ref, qt_ref, ot_ref, z_ref, vok_ref,
            s_ref, h_ref, acc_ref, q8_ref, cs_ref, *, seq, dh):
    f32, bf16 = jnp.float32, jnp.bfloat16
    tq, kc = _TQ, _KC
    nb = _H // _U
    fr = tq // nb
    nw = tq // _W
    kg = _PG * kc
    ng = seq // kg
    ff = w1_ref.shape[1]
    i = pl.program_id(0)
    row0 = pl.multiple_of(i * tq, tq)
    scale = (dh ** -0.5) * math.log2(math.e)

    def rot(r):
        return (r + tq) % seq

    xb = list(_XSPLIT) + [seq]
    nx = len(_XSPLIT)
    x_copies = [
        pltpu.make_async_copy(x_hbm.at[rot(a):rot(a) + b - a],
                              x_ref.at[rot(a):rot(a) + b - a], sems.at[n])
        for n, (a, b) in enumerate(zip(xb[:-1], xb[1:]))]
    w_copies = [
        pltpu.make_async_copy(src, dst, sems.at[nx + n])
        for n, (src, dst) in enumerate(
            [(w1_hbm.at[:, 0:_F0], w1_ref.at[:, 0:_F0]),
             (w1_hbm.at[:, _F0:], w1_ref.at[:, _F0:]),
             (w2_hbm, w2_ref), (wo_hbm, wo_ref)])]
    wq_copies = [
        pltpu.make_async_copy(src, dst, sems.at[nx + 4 + n])
        for n, (src, dst) in enumerate(
            [(wq_hbm, wq_ref), (wkt_hbm, wt_ref.at[0:dh]),
             (wvt_hbm, wt_ref.at[dh:2 * dh])])]

    def prep_queries(qt, a=0, b=tq, hs=range(_H), after=None):
        for h in hs:
            kap = kap_ref[:, a:b]
            if after is not None:
                kap = kap + after(h) * 0.0
            q = qt[h * dh:(h + 1) * dh, :] * kap
            rho = jnp.maximum(
                jnp.max(jnp.abs(q), axis=0, keepdims=True), _TINY)
            qi, dq, qc = _limbs(q * ((16.0 * _QA) * _recip(rho)))
            q8_ref[h * 4 * dh:(h + 1) * 4 * dh, a:b] = jnp.concatenate(
                [qi, qi, dq, qc], axis=0).astype(jnp.int8)
            cs_ref[h:h + 1, a:b] = rho * (1.0 / (_QA * _KA))

    @pl.when(i == 0)
    def _():
        x_copies[0].start()
        for cp in wq_copies:
            cp.start()
        z_ref[...] = jnp.zeros(z_ref.shape, f32)

        def layernorm(n):
            a = n * _LNR
            if a in _XWAIT:
                for c in _XWAIT[a]:
                    x_copies[c].wait()
                if a == 0:
                    for cp in x_copies[1:]:
                        cp.start()
                if a == max(_XWAIT):
                    for cp in w_copies:
                        cp.start()
            a, b = rot(a), rot(a) + _LNR
            x = x_ref[a:b, :].astype(f32)
            mu = jnp.mean(x, axis=-1, keepdims=True)
            xc = x - mu
            var = jnp.mean(xc * xc, axis=-1, keepdims=True)
            xn_ref[a:b, :] = (xc * jax.lax.rsqrt(var + _EPS)).astype(bf16)

        def project(n, want_kv, want_q):
            a, b = rot(n * _LNR), rot(n * _LNR) + _LNR
            lo = 0 if want_kv else 2 * dh
            hi = 2 * dh + (_H * dh if want_q else 0)
            r = jax.lax.dot_general(wt_ref[lo:hi, :], xn_ref[a:b, :], _NT,
                                    preferred_element_type=f32)
            if want_kv:
                kt_ref[:, a:b] = r[0:dh]
                vt_ref[:, a:b] = pltpu.bitcast(
                    r[dh:2 * dh].astype(bf16), jnp.uint32)
            if want_q:
                q = r[2 * dh - lo:]
                qt_ref[a // tq, :, a % tq:a % tq + _LNR] = q
                if b <= tq:
                    prep_queries(q, a, b)

        layernorm(0)
        for cp in wq_copies:
            cp.wait()
        x_copies[1].wait()
        wt_ref[2 * dh:, :] = wq_ref[...].T
        for op, n in _PRO:
            if op == "ln":
                layernorm(n)
            else:
                project(n, "k" in op, "q" in op)

        kt = kt_ref[...]
        kap = jnp.maximum(jnp.max(jnp.abs(kt), axis=1, keepdims=True), _TINY)
        kap_ref[...] = jnp.broadcast_to(kap * scale, kap_ref.shape)
        ki, dk, kcs = _limbs(kt * ((16.0 * _KA) / kap))
        k1 = ki >> 1
        zero = jnp.zeros_like(ki)
        kl = jnp.concatenate([k1, ki - k1, kcs, dk] + [zero] * 4, axis=0)
        for c in range(seq // kc):
            kcl = kl[:, c * kc:(c + 1) * kc].T
            k8_ref[c * kc:(c + 1) * kc, :] = jnp.concatenate(
                [kcl[g * 16:(g + 1) * 16] for g in reversed(range(kc // 16))],
                axis=0).astype(jnp.int8)

        vmax = jnp.max(jnp.abs(pltpu.bitcast(vt_ref[...], bf16).astype(f32)),
                       keepdims=True)
        vok = jnp.logical_and(vmax >= _V_MIN, vmax <= _V_MAX)
        vok_ref[...] = jnp.broadcast_to(jnp.where(vok, 1.0, 0.0), vok_ref.shape)
        for n in _PRO_Q:
            project(n, False, True)
        w_copies[0].wait()

    def heads(j, ok_in):
        q8 = q8_ref[pl.ds(pl.multiple_of(j * (_U * 4 * dh), _U * 4 * dh),
                          _U * 4 * dh), :]
        cs = cs_ref[pl.ds(pl.multiple_of(j * _U, _U), _U), :]
        uw = [(u, w) for u in range(_U) for w in range(nw)]
        l8 = {k: jnp.zeros((8, _W), f32) for k in uw}
        o = {k: z_ref[...] for k in uw}
        ps, outs, oks = {}, {}, {}

        def scores(u, g, w):
            cols = slice(w * _W, (w + 1) * _W)
            t = jnp.dot(k8_ref[g * kg:(g + 1) * kg, 0:4 * dh],
                        q8[u * 4 * dh:(u + 1) * 4 * dh, cols],
                        preferred_element_type=jnp.int32)
            ps[(u, g, w)] = jnp.exp2(t.astype(f32) * cs[u:u + 1, cols])

        def pv(u, g, w):
            pg = ps.pop((u, g, w))
            for e in range(_PG):
                p = pg[e * kc:(e + 1) * kc]
                for r in range(kc // 8):
                    l8[(u, w)] = l8[(u, w)] + p[r * 8:(r + 1) * 8]
                p = jnp.concatenate(
                    [p[n * 16:(n + 1) * 16] for n in reversed(range(kc // 16))],
                    axis=0)
                ks = slice(g * kg + e * kc, g * kg + (e + 1) * kc)
                o[(u, w)] = o[(u, w)] + jnp.dot(
                    pltpu.bitcast(vt_ref[:, ks], bf16), p.astype(bf16),
                    preferred_element_type=f32)
            if g == ng - 1:
                l = jnp.sum(l8[(u, w)], axis=0, keepdims=True)
                outs[(u, w)] = (o[(u, w)] / l).astype(bf16)
                okl = jnp.logical_and(l >= _L_MIN, l <= _L_MAX)
                oks[w] = jnp.logical_and(oks[w], okl) if w in oks else okl

        items = [(u, g, w) for u in range(_U) for g in range(ng)
                 for w in range(nw)]
        for t in range(len(items) + _LAG):
            if t < len(items):
                scores(*items[t])
            if t == len(items):
                rows = pl.ds(pl.multiple_of(row0 + j * fr, fr), fr)
                h_ref[pl.ds(pl.multiple_of(j * fr, fr), fr), :] = _silu(
                    jnp.dot(xn_ref[rows, :], w1_ref[:, 0:_F0],
                            preferred_element_type=f32))
            if t >= _LAG:
                pv(*items[t - _LAG])

        ot_ref[pl.ds(pl.multiple_of(j * (_U * dh), _U * dh), _U * dh), :] = (
            jnp.concatenate(
                [jnp.concatenate([outs[(u, w)] for w in range(nw)], axis=1)
                 for u in range(_U)], axis=0))
        ok = jnp.concatenate(
            [jnp.where(oks[w], 1.0, 0.0) for w in range(nw)], axis=1)
        rho_ok = jnp.max(cs, axis=0, keepdims=True) <= _RHO_MAX / (_QA * _KA)
        return jnp.minimum(ok_in, jnp.where(rho_ok, ok, 0.0))

    ok = jax.lax.fori_loop(0, nb, heads, vok_ref[...])

    @pl.when(i == 0)
    def _():
        for cp in w_copies[1:]:
            cp.wait()

    rows = pl.ds(row0, tq)
    xn = xn_ref[rows, :]
    acc = x_ref[rows, :].astype(f32)
    fedges = [0] + list(range(_F0, ff, _FC)) + [ff]
    fspans = list(zip(fedges[:-1], fedges[1:]))
    assert len(fspans) >= _H // 8 and acc.shape == (tq, tq)

    def hidden(a, b):
        if a == 0:
            return h_ref[...]
        return _silu(jnp.dot(xn, w1_ref[:, a:b], preferred_element_type=f32))

    qn = qt_ref.at[jnp.minimum(i + 1, seq // tq - 1)]
    h_next = hidden(*fspans[0])
    for n, (a, b) in enumerate(fspans):
        h = h_next
        if n + 1 < len(fspans):
            h_next = hidden(*fspans[n + 1])
        acc = acc + jnp.dot(h, w2_ref[a:b, :], preferred_element_type=f32)
        if n < _H // 8:
            prep_queries(qn, hs=range(8 * n, 8 * n + 8),
                         after=lambda h: acc[(h % 8) * 64:(h % 8) * 64 + 1, :])
    acc_ref[...] = acc
    o_ref[...] = (acc + jax.lax.dot_general(
        ot_ref[...], wo_ref[...], _TN,
        preferred_element_type=f32)).astype(o_ref.dtype)

    @pl.when(jnp.min(ok) < 0.5)
    def _():
        def safe_head(h, carry):
            hr = pl.ds(pl.multiple_of(h * dh, dh), dh)
            q = (qt_ref[i, hr, :] * scale).astype(bf16)

            def pass1(c, m8):
                ks = pl.ds(pl.multiple_of(c * _SC, _SC), _SC)
                s = jax.lax.dot_general(kt_ref[:, ks].astype(bf16), q, _TN,
                                        preferred_element_type=f32)
                s_ref[ks, :] = s
                return jnp.maximum(
                    m8, jnp.max(s.reshape(_SC // 8, 8, tq), axis=0))

            m8 = jax.lax.fori_loop(0, seq // _SC, pass1,
                                   jnp.full((8, tq), -jnp.inf, f32))
            m = jnp.max(m8, axis=0, keepdims=True)

            def pass2(c, lo):
                ks = pl.ds(pl.multiple_of(c * _SC, _SC), _SC)
                p = jnp.exp2(s_ref[ks, :] - m)
                return (lo[0] + jnp.sum(p.reshape(_SC // 8, 8, tq), axis=0),
                        lo[1] + jnp.dot(pltpu.bitcast(vt_ref[:, ks], bf16),
                                        p.astype(bf16),
                                        preferred_element_type=f32))

            l8, o = jax.lax.fori_loop(
                0, seq // _SC, pass2,
                (jnp.zeros((8, tq), f32), jnp.zeros((dh, tq), f32)))
            l = jnp.sum(l8, axis=0, keepdims=True)
            ot_ref[hr, :] = (o / l).astype(bf16)
            return carry

        jax.lax.fori_loop(0, _H, safe_head, 0)

        def redo_out(r, carry):
            rs = pl.ds(pl.multiple_of(r * 128, 128), 128)
            o_ref[rs, :] = (acc_ref[rs, :] + jax.lax.dot_general(
                ot_ref[:, rs], wo_ref[...], _TN,
                preferred_element_type=f32)).astype(o_ref.dtype)
            return carry

        jax.lax.fori_loop(0, tq // 128, redo_out, 0)


@jax.jit
def pallas_parallel_sum__grouped_kv_mqa__dense_activation_silu__prompt_kernel(
    A_x: jax.Array,
    A_wq: jax.Array,
    A_wk: jax.Array,
    A_wv: jax.Array,
    A_wo: jax.Array,
    B_x: jax.Array,
    B_w1: jax.Array,
    B_w2: jax.Array,
):
    del B_x
    b, seq, d = A_x.shape
    dh = A_wk.shape[1]
    ff = B_w1.shape[1]
    hd = _H * dh
    assert b == 1 and seq == 8 * _LNR == 4 * _TQ and dh == 16
    assert A_wq.shape == (d, hd) and ff % 128 == 0
    bf16, f32 = jnp.bfloat16, jnp.float32

    out = pl.pallas_call(
        functools.partial(_kernel, seq=seq, dh=dh),
        grid=(seq // _TQ,),
        in_specs=[pl.BlockSpec(memory_space=pl.ANY)] * 7,
        out_specs=pl.BlockSpec((_TQ, d), lambda i: (i, 0)),
        out_shape=jax.ShapeDtypeStruct((seq, d), A_x.dtype),
        scratch_shapes=[
            pltpu.VMEM((seq, d), bf16),
            pltpu.VMEM((d, hd), bf16),
            pltpu.VMEM((hd, d), bf16),
            pltpu.VMEM((d, ff), bf16),
            pltpu.VMEM((ff, d), bf16),
            pltpu.SemaphoreType.DMA((len(_XSPLIT) + 7,)),
            pltpu.VMEM((hd + 2 * dh, d), bf16),
            pltpu.VMEM((dh, seq), f32),
            pltpu.VMEM((seq, d), bf16),
            pltpu.VMEM((seq, 128), jnp.int8),
            pltpu.VMEM((dh, _TQ), f32),
            pltpu.VMEM((dh // 2, seq), jnp.uint32),
            pltpu.VMEM((seq // _TQ, hd, _TQ), f32),
            pltpu.VMEM((hd, _TQ), bf16),
            pltpu.VMEM((dh, _W), f32),
            pltpu.VMEM((1, _TQ), f32),
            pltpu.VMEM((seq, _TQ), f32),
            pltpu.VMEM((_TQ, _F0), bf16),
            pltpu.VMEM((_TQ, d), f32),
            pltpu.VMEM((4 * hd, _TQ), jnp.int8),
            pltpu.VMEM((_H, _TQ), f32),
        ],
        compiler_params=pltpu.CompilerParams(
            dimension_semantics=("arbitrary",),
            vmem_limit_bytes=64 * 1024 * 1024,
        ),
    )(A_x.reshape(seq, d), A_wq, A_wk.T, A_wv.T, A_wo, B_w1, B_w2)
    return out.reshape(b, seq, d)
```

```python
import functools
import math

import jax
import jax.numpy as jnp
from jax.experimental import pallas as pl
from jax.experimental.pallas import tpu as pltpu

_H = 32
_EPS = 1e-5
_TQ = 512
_KC = 128
_PG = 2
_W = 256
_LAG = 3
_U = 16
_F0 = 128
_FC = 512
_SC = 256
_NO = 2
_LNR = 256

_QA, _KA = 127.0, 254.0
_TINY = 1e-30
_RHO_MAX = 32.0
_L_MIN, _L_MAX = 2.0 ** -40, 2.0 ** 64
_V_MIN, _V_MAX = 2.0 ** -30, 2.0 ** 60

_XSPLIT = (0, 256, 512, 1024, 1536)
_XWAIT = {0: (0,), 512: (2,), 1024: (3, 4)}
_PRO = (("ln", 1), ("kq", 0), ("ln", 2), ("kq", 1), ("ln", 3), ("kq", 2),
        ("ln", 4), ("ln", 5), ("kq", 3), ("ln", 6), ("ln", 7), ("kq", 4),
        ("k", 6), ("k", 7), ("kq", 5))
_PRO_Q = (6, 7)

_NT = (((1,), (1,)), ((), ()))
_TN = (((0,), (0,)), ((), ()))


def _limbs(t16):
    b = pltpu.bitcast(t16 + (12582912.0 + 8.0), jnp.int32)
    return b >> 4, (b & 15) - 8, (b + 120) >> 8


def _recip(x):
    r = pl.reciprocal(x, approx=True)
    return r * (2.0 - x * r)


def _silu(h):
    return (h * jax.nn.sigmoid(h)).astype(jnp.bfloat16)


def _kernel(x_hbm, wq_hbm, wkt_hbm, wvt_hbm, wo_hbm, w1_hbm, w2_hbm, o_hbm,
            x_ref, wq_ref, wo_ref, w1_ref, w2_ref, sems, wt_ref, kt_ref,
            xn_ref, k8_ref, kap_ref, vt_ref, qt_ref, ot_ref, z_ref, vok_ref,
            s_ref, h_ref, acc_ref, q8_ref, cs_ref, o_ref, osems, *, seq, dh):
    f32, bf16 = jnp.float32, jnp.bfloat16
    tq, kc = _TQ, _KC
    nb = _H // _U
    fr = tq // nb
    nw = tq // _W
    kg = _PG * kc
    ng = seq // kg
    ff = w1_ref.shape[1]
    i = pl.program_id(0)
    row0 = pl.multiple_of(i * tq, tq)
    scale = (dh ** -0.5) * math.log2(math.e)

    def rot(r):
        return (r + tq) % seq

    xb = list(_XSPLIT) + [seq]
    nx = len(_XSPLIT)
    x_copies = [
        pltpu.make_async_copy(x_hbm.at[rot(a):rot(a) + b - a],
                              x_ref.at[rot(a):rot(a) + b - a], sems.at[n])
        for n, (a, b) in enumerate(zip(xb[:-1], xb[1:]))]
    w_copies = [
        pltpu.make_async_copy(src, dst, sems.at[nx + n])
        for n, (src, dst) in enumerate(
            [(w1_hbm.at[:, 0:_F0], w1_ref.at[:, 0:_F0]),
             (w1_hbm.at[:, _F0:], w1_ref.at[:, _F0:]),
             (w2_hbm, w2_ref), (wo_hbm, wo_ref)])]
    wq_copies = [
        pltpu.make_async_copy(src, dst, sems.at[nx + 4 + n])
        for n, (src, dst) in enumerate(
            [(wq_hbm, wq_ref), (wkt_hbm, wt_ref.at[0:dh]),
             (wvt_hbm, wt_ref.at[dh:2 * dh])])]

    def prep_queries(qt, a=0, b=tq, hs=range(_H), after=None):
        for h in hs:
            kap = kap_ref[:, a:b]
            if after is not None:
                kap = kap + after(h) * 0.0
            q = qt[h * dh:(h + 1) * dh, :] * kap
            rho = jnp.maximum(
                jnp.max(jnp.abs(q), axis=0, keepdims=True), _TINY)
            qi, dq, qc = _limbs(q * ((16.0 * _QA) * _recip(rho)))
            q8_ref[h * 4 * dh:(h + 1) * 4 * dh, a:b] = jnp.concatenate(
                [qi, qi, dq, qc], axis=0).astype(jnp.int8)
            cs_ref[h:h + 1, a:b] = rho * (1.0 / (_QA * _KA))

    @pl.when(i == 0)
    def _():
        x_copies[0].start()
        for cp in wq_copies:
            cp.start()
        z_ref[...] = jnp.zeros(z_ref.shape, f32)

        def layernorm(n):
            a = n * _LNR
            if a in _XWAIT:
                for c in _XWAIT[a]:
                    x_copies[c].wait()
                if a == 0:
                    for cp in x_copies[1:]:
                        cp.start()
                if a == max(_XWAIT):
                    for cp in w_copies:
                        cp.start()
            a, b = rot(a), rot(a) + _LNR
            x = x_ref[a:b, :].astype(f32)
            mu = jnp.mean(x, axis=-1, keepdims=True)
            xc = x - mu
            var = jnp.mean(xc * xc, axis=-1, keepdims=True)
            xn_ref[a:b, :] = (xc * jax.lax.rsqrt(var + _EPS)).astype(bf16)

        def project(n, want_kv, want_q):
            a, b = rot(n * _LNR), rot(n * _LNR) + _LNR
            lo = 0 if want_kv else 2 * dh
            hi = 2 * dh + (_H * dh if want_q else 0)
            r = jax.lax.dot_general(wt_ref[lo:hi, :], xn_ref[a:b, :], _NT,
                                    preferred_element_type=f32)
            if want_kv:
                kt_ref[:, a:b] = r[0:dh]
                vt_ref[:, a:b] = pltpu.bitcast(
                    r[dh:2 * dh].astype(bf16), jnp.uint32)
            if want_q:
                q = r[2 * dh - lo:]
                qt_ref[a // tq, :, a % tq:a % tq + _LNR] = q
                if b <= tq:
                    prep_queries(q, a, b)

        layernorm(0)
        for cp in wq_copies:
            cp.wait()
        x_copies[1].wait()
        wt_ref[2 * dh:, :] = wq_ref[...].T
        for op, n in _PRO:
            if op == "ln":
                layernorm(n)
            else:
                project(n, "k" in op, "q" in op)

        kt = kt_ref[...]
        kap = jnp.maximum(jnp.max(jnp.abs(kt), axis=1, keepdims=True), _TINY)
        kap_ref[...] = jnp.broadcast_to(kap * scale, kap_ref.shape)
        ki, dk, kcs = _limbs(kt * ((16.0 * _KA) / kap))
        k1 = ki >> 1
        zero = jnp.zeros_like(ki)
        kl = jnp.concatenate([k1, ki - k1, kcs, dk] + [zero] * 4, axis=0)
        for c in range(seq // kc):
            kcl = kl[:, c * kc:(c + 1) * kc].T
            k8_ref[c * kc:(c + 1) * kc, :] = jnp.concatenate(
                [kcl[g * 16:(g + 1) * 16] for g in reversed(range(kc // 16))],
                axis=0).astype(jnp.int8)

        vmax = jnp.max(jnp.abs(pltpu.bitcast(vt_ref[...], bf16).astype(f32)),
                       keepdims=True)
        vok = jnp.logical_and(vmax >= _V_MIN, vmax <= _V_MAX)
        vok_ref[...] = jnp.broadcast_to(jnp.where(vok, 1.0, 0.0), vok_ref.shape)
        for n in _PRO_Q:
            project(n, False, True)
        w_copies[0].wait()

    oc = tq // _NO

    def out_copy(r, base):
        return pltpu.make_async_copy(
            o_ref.at[r * oc:(r + 1) * oc],
            o_hbm.at[pl.ds(pl.multiple_of(base + r * oc, oc), oc)], osems.at[r])

    def heads(j, ok_in):
        q8 = q8_ref[pl.ds(pl.multiple_of(j * (_U * 4 * dh), _U * 4 * dh),
                          _U * 4 * dh), :]
        cs = cs_ref[pl.ds(pl.multiple_of(j * _U, _U), _U), :]
        uw = [(u, w) for u in range(_U) for w in range(nw)]
        l8 = {k: jnp.zeros((8, _W), f32) for k in uw}
        o = {k: z_ref[...] for k in uw}
        ps, outs, oks = {}, {}, {}

        def scores(u, g, w):
            cols = slice(w * _W, (w + 1) * _W)
            t = jnp.dot(k8_ref[g * kg:(g + 1) * kg, 0:4 * dh],
                        q8[u * 4 * dh:(u + 1) * 4 * dh, cols],
                        preferred_element_type=jnp.int32)
            ps[(u, g, w)] = jnp.exp2(t.astype(f32) * cs[u:u + 1, cols])

        def pv(u, g, w):
            pg = ps.pop((u, g, w))
            for e in range(_PG):
                p = pg[e * kc:(e + 1) * kc]
                for r in range(kc // 8):
                    l8[(u, w)] = l8[(u, w)] + p[r * 8:(r + 1) * 8]
                p = jnp.concatenate(
                    [p[n * 16:(n + 1) * 16] for n in reversed(range(kc // 16))],
                    axis=0)
                ks = slice(g * kg + e * kc, g * kg + (e + 1) * kc)
                o[(u, w)] = o[(u, w)] + jnp.dot(
                    pltpu.bitcast(vt_ref[:, ks], bf16), p.astype(bf16),
                    preferred_element_type=f32)
            if g == ng - 1:
                l = jnp.sum(l8[(u, w)], axis=0, keepdims=True)
                outs[(u, w)] = (o[(u, w)] / l).astype(bf16)
                okl = jnp.logical_and(l >= _L_MIN, l <= _L_MAX)
                oks[w] = jnp.logical_and(oks[w], okl) if w in oks else okl

        items = [(u, g, w) for u in range(_U) for g in range(ng)
                 for w in range(nw)]
        for t in range(len(items) + _LAG):
            if t < len(items):
                scores(*items[t])
            if t == len(items):
                rows = pl.ds(pl.multiple_of(row0 + j * fr, fr), fr)
                h_ref[pl.ds(pl.multiple_of(j * fr, fr), fr), :] = _silu(
                    jnp.dot(xn_ref[rows, :], w1_ref[:, 0:_F0],
                            preferred_element_type=f32))
            if t >= _LAG:
                pv(*items[t - _LAG])

        ot_ref[pl.ds(pl.multiple_of(j * (_U * dh), _U * dh), _U * dh), :] = (
            jnp.concatenate(
                [jnp.concatenate([outs[(u, w)] for w in range(nw)], axis=1)
                 for u in range(_U)], axis=0))
        ok = jnp.concatenate(
            [jnp.where(oks[w], 1.0, 0.0) for w in range(nw)], axis=1)
        rho_ok = jnp.max(cs, axis=0, keepdims=True) <= _RHO_MAX / (_QA * _KA)
        return jnp.minimum(ok_in, jnp.where(rho_ok, ok, 0.0))

    ok = jax.lax.fori_loop(0, nb, heads, vok_ref[...])

    @pl.when(i == 0)
    def _():
        for cp in w_copies[1:]:
            cp.wait()

    @pl.when(i > 0)
    def _():
        for r in range(_NO):
            out_copy(r, row0 - tq).wait()

    rows = pl.ds(row0, tq)
    xn = xn_ref[rows, :]
    acc = x_ref[rows, :].astype(f32)
    fedges = [0] + list(range(_F0, ff, _FC)) + [ff]
    fspans = list(zip(fedges[:-1], fedges[1:]))
    assert len(fspans) >= _H // 8 and acc.shape == (tq, tq)

    def hidden(a, b):
        if a == 0:
            return h_ref[...]
        return _silu(jnp.dot(xn, w1_ref[:, a:b], preferred_element_type=f32))

    qn = qt_ref.at[jnp.minimum(i + 1, seq // tq - 1)]
    h_next = hidden(*fspans[0])
    for n, (a, b) in enumerate(fspans):
        h = h_next
        if n + 1 < len(fspans):
            h_next = hidden(*fspans[n + 1])
        acc = acc + jnp.dot(h, w2_ref[a:b, :], preferred_element_type=f32)
        if n < _H // 8:
            prep_queries(qn, hs=range(8 * n, 8 * n + 8),
                         after=lambda h: acc[(h % 8) * 64:(h % 8) * 64 + 1, :])
    acc_ref[...] = acc
    for r in range(_NO):
        rs = slice(r * oc, (r + 1) * oc)
        o_ref[rs, :] = (acc[rs] + jax.lax.dot_general(
            ot_ref[:, rs], wo_ref[...], _TN,
            preferred_element_type=f32)).astype(o_ref.dtype)
        out_copy(r, row0).start()

    @pl.when(jnp.min(ok) < 0.5)
    def _():
        def safe_head(h, carry):
            hr = pl.ds(pl.multiple_of(h * dh, dh), dh)
            q = (qt_ref[i, hr, :] * scale).astype(bf16)

            def pass1(c, m8):
                ks = pl.ds(pl.multiple_of(c * _SC, _SC), _SC)
                s = jax.lax.dot_general(kt_ref[:, ks].astype(bf16), q, _TN,
                                        preferred_element_type=f32)
                s_ref[ks, :] = s
                return jnp.maximum(
                    m8, jnp.max(s.reshape(_SC // 8, 8, tq), axis=0))

            m8 = jax.lax.fori_loop(0, seq // _SC, pass1,
                                   jnp.full((8, tq), -jnp.inf, f32))
            m = jnp.max(m8, axis=0, keepdims=True)

            def pass2(c, lo):
                ks = pl.ds(pl.multiple_of(c * _SC, _SC), _SC)
                p = jnp.exp2(s_ref[ks, :] - m)
                return (lo[0] + jnp.sum(p.reshape(_SC // 8, 8, tq), axis=0),
                        lo[1] + jnp.dot(pltpu.bitcast(vt_ref[:, ks], bf16),
                                        p.astype(bf16),
                                        preferred_element_type=f32))

            l8, o = jax.lax.fori_loop(
                0, seq // _SC, pass2,
                (jnp.zeros((8, tq), f32), jnp.zeros((dh, tq), f32)))
            l = jnp.sum(l8, axis=0, keepdims=True)
            ot_ref[hr, :] = (o / l).astype(bf16)
            return carry

        jax.lax.fori_loop(0, _H, safe_head, 0)
        for r in range(_NO):
            out_copy(r, row0).wait()

        def redo_out(r, carry):
            rs = pl.ds(pl.multiple_of(r * 128, 128), 128)
            o_ref[rs, :] = (acc_ref[rs, :] + jax.lax.dot_general(
                ot_ref[:, rs], wo_ref[...], _TN,
                preferred_element_type=f32)).astype(o_ref.dtype)
            return carry

        jax.lax.fori_loop(0, tq // 128, redo_out, 0)
        for r in range(_NO):
            out_copy(r, row0).start()

    @pl.when(i == seq // tq - 1)
    def _():
        for r in range(_NO):
            out_copy(r, row0).wait()


@jax.jit
def pallas_parallel_sum__grouped_kv_mqa__dense_activation_silu__prompt_kernel(
    A_x: jax.Array,
    A_wq: jax.Array,
    A_wk: jax.Array,
    A_wv: jax.Array,
    A_wo: jax.Array,
    B_x: jax.Array,
    B_w1: jax.Array,
    B_w2: jax.Array,
):
    del B_x
    b, seq, d = A_x.shape
    dh = A_wk.shape[1]
    ff = B_w1.shape[1]
    hd = _H * dh
    assert b == 1 and seq == 8 * _LNR == 4 * _TQ and dh == 16
    assert A_wq.shape == (d, hd) and ff % 128 == 0
    bf16, f32 = jnp.bfloat16, jnp.float32

    out = pl.pallas_call(
        functools.partial(_kernel, seq=seq, dh=dh),
        grid=(seq // _TQ,),
        in_specs=[pl.BlockSpec(memory_space=pl.ANY)] * 7,
        out_specs=pl.BlockSpec(memory_space=pl.ANY),
        out_shape=jax.ShapeDtypeStruct((seq, d), A_x.dtype),
        scratch_shapes=[
            pltpu.VMEM((seq, d), bf16),
            pltpu.VMEM((d, hd), bf16),
            pltpu.VMEM((hd, d), bf16),
            pltpu.VMEM((d, ff), bf16),
            pltpu.VMEM((ff, d), bf16),
            pltpu.SemaphoreType.DMA((len(_XSPLIT) + 7,)),
            pltpu.VMEM((hd + 2 * dh, d), bf16),
            pltpu.VMEM((dh, seq), f32),
            pltpu.VMEM((seq, d), bf16),
            pltpu.VMEM((seq, 128), jnp.int8),
            pltpu.VMEM((dh, _TQ), f32),
            pltpu.VMEM((dh // 2, seq), jnp.uint32),
            pltpu.VMEM((seq // _TQ, hd, _TQ), f32),
            pltpu.VMEM((hd, _TQ), bf16),
            pltpu.VMEM((dh, _W), f32),
            pltpu.VMEM((1, _TQ), f32),
            pltpu.VMEM((seq, _TQ), f32),
            pltpu.VMEM((_TQ, _F0), bf16),
            pltpu.VMEM((_TQ, d), f32),
            pltpu.VMEM((4 * hd, _TQ), jnp.int8),
            pltpu.VMEM((_H, _TQ), f32),
            pltpu.VMEM((_TQ, d), bf16),
            pltpu.SemaphoreType.DMA((_NO,)),
        ],
        compiler_params=pltpu.CompilerParams(
            dimension_semantics=("arbitrary",),
            vmem_limit_bytes=64 * 1024 * 1024,
        ),
    )(A_x.reshape(seq, d), A_wq, A_wk.T, A_wv.T, A_wo, B_w1, B_w2)
    return out.reshape(b, seq, d)
```
